```python
import jax
import jax.numpy as jnp

def _softmax(x, axis=-1):
    return jax.nn.softmax(x, axis=axis)

def _gelu(x):
    return jax.nn.gelu(x, approximate=True)

def _silu(x):
    return jax.nn.silu(x)

def _sigmoid(x):
    return jax.nn.sigmoid(x)

def _layernorm(x, axis=-1, eps=1e-05):
    m = jnp.mean(x, axis=axis, keepdims=True)
    v = jnp.var(x, axis=axis, keepdims=True)
    return (x - m) / jnp.sqrt(v + eps)

def _scatter_add(tgt, idx, src, axis=0):
    return tgt.at[idx].add(src)

def _segment_sum(src, seg, n):
    return jax.ops.segment_sum(src, seg, n)

class _Rng:

    def __init__(self, key):
        self._k = key

    def _next(self):
        self._k, sub = jax.random.split(self._k)
        return sub

    def normal(self, shape):
        return jax.random.normal(self._next(), shape, dtype=jnp.bfloat16)

    def randint(self, lo, hi, shape):
        return jax.random.randint(self._next(), shape, lo, hi, dtype=jnp.int32)

    def uniform(self, shape, lo=0.0, hi=1.0):
        return jax.random.uniform(self._next(), shape, jnp.bfloat16, lo, hi)

    def permutation(self, n):
        return jax.random.permutation(self._next(), n)
kernel_name = 'standalone__conformer_family_branchformer__speech'

def setup_inputs():
    _rng = _Rng(jax.random.key(int.from_bytes(__import__("os").urandom(4), "little")))
    _w = lambda a: (lambda t: t.astype(jnp.bfloat16) if jnp.issubdtype(t.dtype, jnp.floating) else t)(jnp.asarray(a))
    B, T, D, K = (2, 4000, 512, 31)
    s = float(D) ** (-0.5)
    return {'x': _w((lambda *s: _rng.normal(s) * 0.05)(B, T, D)), 'w_q': _w((lambda *s: _rng.normal(s) * 0.05)(D, D) * s), 'w_k': _w((lambda *s: _rng.normal(s) * 0.05)(D, D) * s), 'w_v': _w((lambda *s: _rng.normal(s) * 0.05)(D, D) * s), 'w_ao': _w((lambda *s: _rng.normal(s) * 0.05)(D, D) * s), 'w_up': _w((lambda *s: _rng.normal(s) * 0.05)(D, 2 * D) * s), 'dw': _w((lambda *s: _rng.normal(s) * 0.05)(K, D) * (1.0 / K)), 'w_dn': _w((lambda *s: _rng.normal(s) * 0.05)(D, D) * s), 'w_merge': _w((lambda *s: _rng.normal(s) * 0.05)(2 * D, D) * s)}

def reference(x, w_q, w_k, w_v, w_ao, w_up, dw, w_dn, w_merge):
    B, T, D = x.shape
    K = dw.shape[0]
    xa = _layernorm(x, axis=-1)
    q = jnp.einsum('btd,de->bte', xa, w_q)
    k = jnp.einsum('btd,de->bte', xa, w_k)
    v = jnp.einsum('btd,de->bte', xa, w_v)
    logits = jnp.einsum('btd,bsd->bts', q, k) * float(D) ** (-0.5)
    attn = _softmax(logits, axis=-1)
    ya = jnp.einsum('bts,bsd->btd', attn, v)
    ya = jnp.einsum('btd,de->bte', ya, w_ao)
    xc = _layernorm(x, axis=-1)
    h = _gelu(jnp.einsum('btd,de->bte', xc, w_up))
    u = h[..., :D].copy()
    g = _layernorm(h[..., D:], axis=-1)
    pad = K // 2
    gp = jnp.pad(g, ((0, 0), (pad, pad), (0, 0)))
    conv = jnp.zeros_like(g)
    for i in range(K):
        conv = conv + gp[:, i:i + T, :] * dw[i][None, None, :]
    yc = jnp.einsum('btd,de->bte', u * conv, w_dn)
    merged = jnp.concatenate([ya, yc], axis=-1)
    out = jnp.einsum('btf,fd->btd', merged, w_merge)
    return x + out
```

```python
import functools
import math

import jax
import jax.numpy as jnp
import numpy as np
from jax import lax
import jax.experimental.pallas as pl
import jax.experimental.pallas.tpu as pltpu

F32 = jnp.float32
BF16 = jnp.bfloat16
EPS = 1e-5
LOG2E = 1.4426950408889634
HALO = 16
LN = 128


def _ln(x):
    m = jnp.mean(x, axis=-1, keepdims=True)
    xc = x - m
    v = jnp.mean(xc * xc, axis=-1, keepdims=True)
    return xc * lax.rsqrt(v + EPS)


def _gelu(x):
    c = math.sqrt(2.0 / math.pi)
    return (0.5 * x) * (1.0 + jnp.tanh(x * (c + (c * 0.044715) * (x * x))))


def _dot(a, b):
    return jnp.dot(a, b, preferred_element_type=F32)


def _dot_nt(a, b):
    return lax.dot_general(a, b, (((1,), (1,)), ((), ())), preferred_element_type=F32)


def _cat(xs):
    return jnp.concatenate(xs, axis=1)


def _spread(o, n):
    g = o.shape[0] // 8
    k = n // 8
    return jnp.concatenate([o[8 * (i * g // k):8 * (i * g // k) + 8] for i in range(k)], axis=0)


def make(TQ=400, LNT=3, flags=None):
    KC = 512

    def kernel(x_ref, wq_ref, wk_ref, wv_ref, wao_ref, wup_ref, dw_ref, wdn_ref, wm_ref,
               o_ref,
               wqk_s, wout_s, xa_s, dwb_s, z_s,
               g_s, cv_s, q_s, h_s, m_s, l_s, ya_s, yc_s, o_s, s_s, p_s, acc_s,
               *, T, D, K, TP):
        b = pl.program_id(0)
        i = pl.program_id(1)
        NCH = TP // KC
        ND = D // LN
        NT = KC // LN
        NKT = TP // LN
        lt = lambda c: slice(c * LN, (c + 1) * LN)

        @pl.when((b == 0) & (i == 0))
        def _():
            scale = float(D) ** -0.5 * LOG2E
            wqk_s[...] = (_dot_nt(wq_ref[...], wk_ref[...]) * scale).astype(BF16)
            t = _dot(wao_ref[...], wm_ref[0:D, :]).astype(BF16)
            wout_s[D:2 * D, :] = _dot(wdn_ref[...], wm_ref[D:2 * D, :]).astype(BF16)
            wout_s[0:D, :] = _dot(wv_ref[...], t).astype(BF16)
            xa_s[:, T:TP, :] = jnp.zeros((ND, TP - T, LN), BF16)
            z_s[0] = 0
            dw = dw_ref[...].astype(F32)
            for k in range(K):
                dwb_s[k] = jnp.broadcast_to(dw[k:k + 1, :], (8, D))
            for ref in (g_s, cv_s, q_s, h_s, m_s, l_s, ya_s, yc_s, o_s, s_s, p_s, acc_s):
                ref[b, 0:16, :] = jnp.zeros((16, LN), ref.dtype)

        @pl.when(i == 0)
        def _():
            def body(j, c):
                r0 = pl.multiple_of(j * TQ, 16)
                xa = _ln(x_ref[pl.ds(r0, TQ), :].astype(F32))
                for c_ in range(ND):
                    xa_s[c_, pl.ds(r0, TQ), :] = xa[:, lt(c_)].astype(BF16)
                return c
            lax.fori_loop(0, T // TQ, body, 0)
            x0 = _cat([xa_s[c, 0:HALO, :] for c in range(ND)])
            g0 = _ln(_gelu(_dot(x0, wup_ref[:, D:2 * D])))
            for c in range(ND):
                g_s[c, TQ:TQ + HALO, :] = jnp.zeros((HALO, LN), F32)
                g_s[c, TQ + HALO:TQ + 2 * HALO, :] = g0[:, lt(c)]

        r0 = pl.multiple_of(i * TQ, 16)
        never = lax.broadcasted_iota(jnp.int32, (8, LN), 1) < z_s[0]

        def after(v, o):
            n = v.shape[0]
            if o.shape[0] != n:
                o = _spread(o, n)
            return jnp.where(never[None], o.reshape(n // 8, 8, LN), v.reshape(n // 8, 8, LN)).reshape(n, LN)

        xrows = lambda r: _cat([xa_s[c, pl.ds(r, TQ), :] for c in range(ND)])
        ld4 = lambda ref, c0=0: _cat([ref[c0 + c] for c in range(ND)])

        for c in range(ND):
            qc = _dot(xrows(r0), wqk_s[:, lt(c)])
            if c == 0:
                qc = after(qc, jnp.zeros_like(qc))
            q_s[c] = qc.astype(BF16)
            g_s[c, 0:2 * HALO, :] = after(g_s[c, TQ:TQ + 2 * HALO, :], qc)

        for c in range(ND):
            h_s[c] = _gelu(_dot(xrows(r0 + HALO), wup_ref[:, lt(ND + c)]))

        def gate_norm(a0, n, o):
            hs = [h_s[c, a0:a0 + n, :] for c in range(ND)]
            gg = _ln(_cat(hs))
            for c in range(ND):
                gc = after(gg[:, lt(c)], o)
                if a0 + n == TQ:
                    row = lax.broadcasted_iota(jnp.int32, (HALO, LN), 0) + (r0 + TQ)
                    g_s[c, 2 * HALO + a0:HALO + TQ, :] = gc[0:n - HALO]
                    g_s[c, HALO + TQ:2 * HALO + TQ, :] = jnp.where(row < T, gc[n - HALO:n], 0.0)
                else:
                    g_s[c, 2 * HALO + a0:2 * HALO + a0 + n, :] = gc

        def conv_part(c, a0, rc, o):
            gt = g_s[c, a0:a0 + rc + 2 * HALO, :].reshape((rc + 2 * HALO) // 8, 8, LN)
            acc = None
            for bb in range(8):
                n = rc // 8 + (1 if bb else 0)
                y = None
                for a in range(4):
                    k = 8 * a + bb - 1
                    if k < 0:
                        continue
                    t = gt[a:a + n] * dwb_s[k, :, lt(c)][None]
                    y = t if y is None else y + t
                y = y.reshape(n * 8, LN)[bb:bb + rc]
                acc = y if acc is None else acc + y
            cv_s[c, a0:a0 + rc, :] = after(acc, o)

        def local_branch(c):
            u = _gelu(_dot(xrows(r0), wup_ref[:, lt(c)]))
            yc_s[c] = (u * cv_s[c]).astype(BF16)
            o = _dot(yc_s[c], wout_s[D + c * LN:D + (c + 1) * LN, :])
            for n in range(ND):
                base = x_ref[pl.ds(r0, TQ), lt(n)].astype(F32) if c == 0 else o_s[n]
                o_s[n] = o[:, lt(n)] + base

        ends = [LNT + (c + 1) * (NKT - LNT) // ND for c in range(ND)]
        starts = [LNT] + ends[:-1]
        for kt in range(NKT):
            s = _dot_nt(ld4(q_s), _cat([xa_s[d, lt(kt), :] for d in range(ND)]))
            if (kt + 1) * LN > T:
                col = lax.broadcasted_iota(jnp.int32, s.shape, 1) + kt * LN
                s = jnp.where(col < T, s, -jnp.inf)
            s_s[kt] = s
            m = s if kt == 0 else jnp.maximum(s, m_s[0])
            if kt + 1 == NKT:
                m = jnp.broadcast_to(jnp.max(m, axis=-1, keepdims=True), (TQ, LN))
            m_s[0] = m
            if kt < LNT:
                e0, e1 = [8 * (p * (TQ // 8) // LNT) for p in (kt, kt + 1)]
                gate_norm(e0, e1 - e0, s)
            for c in range(ND):
                if starts[c] <= kt < ends[c]:
                    np_ = ends[c] - starts[c]
                    e0, e1 = [8 * (p * (TQ // 8) // np_) for p in (kt - starts[c], kt - starts[c] + 1)]
                    conv_part(c, e0, e1 - e0, s)
                if kt + 1 == ends[c]:
                    local_branch(c)

        def exp_tile(kt, o):
            p = jnp.exp2(s_s[kt] - m_s[0])
            if o is not None:
                p = after(p, o)
            p_s[kt] = p.astype(BF16)
            l = p if kt == 0 else p + l_s[0]
            if kt + 1 == NKT:
                l = jnp.broadcast_to(1.0 / jnp.sum(l, axis=-1, keepdims=True), (TQ, LN))
            l_s[0] = l

        for kt in range(5):
            exp_tile(kt, None)
        for j in range(NCH):
            for c in range(ND):
                o = _dot(ld4(p_s, j * NT), xa_s[c, j * KC:(j + 1) * KC, :])
                if j * NT + c + 5 < NKT:
                    exp_tile(j * NT + c + 5, o)
                if j > 0:
                    o = o + acc_s[c]
                if j < NCH - 1:
                    acc_s[c] = o
                else:
                    ya_s[c] = (o * l_s[0]).astype(BF16)
        for c in range(ND):
            o_ref[:, lt(c)] = (_dot(ld4(ya_s), wout_s[0:D, lt(c)]) + o_s[c]).astype(o_ref.dtype)

    @jax.jit
    def fn(x, w_q, w_k, w_v, w_ao, w_up, dw, w_dn, w_merge):
        B, T, D = x.shape
        K = dw.shape[0]
        TP = (T + KC - 1) // KC * KC
        NKT = TP // LN
        ND = D // LN
        full = lambda a: pl.BlockSpec(a.shape, lambda b, i: (0,) * a.ndim)
        V = pltpu.VMEM
        return pl.pallas_call(
            functools.partial(kernel, T=T, D=D, K=K, TP=TP),
            grid=(B, T // TQ),
            in_specs=[pl.BlockSpec((None, T, D), lambda b, i: (b, 0, 0))]
            + [full(a) for a in (w_q, w_k, w_v, w_ao, w_up, dw, w_dn, w_merge)],
            out_specs=pl.BlockSpec((None, TQ, D), lambda b, i: (b, i, 0)),
            out_shape=jax.ShapeDtypeStruct(x.shape, x.dtype),
            scratch_shapes=[
                V((D, D), BF16),
                V((2 * D, D), BF16),
                V((ND, TP, LN), BF16),
                V((K, 8, D), F32),
                pltpu.SMEM((1,), jnp.int32),
                V((ND, TQ + 2 * HALO, LN), F32),
                V((ND, TQ, LN), F32),
                V((ND, TQ, LN), BF16),
                V((ND, TQ, LN), F32),
                V((1, TQ, LN), F32),
                V((1, TQ, LN), F32),
                V((ND, TQ, LN), BF16),
                V((ND, TQ, LN), BF16),
                V((ND, TQ, LN), F32),
                V((NKT, TQ, LN), F32),
                V((NKT, TQ, LN), BF16),
                V((ND, TQ, LN), F32),
            ],
            compiler_params=pltpu.CompilerParams(
                dimension_semantics=("arbitrary", "arbitrary"),
                vmem_limit_bytes=100 * 1024 * 1024,
                flags=flags,
            ),
        )(x, w_q, w_k, w_v, w_ao, w_up, dw, w_dn, w_merge)

    return fn


_KERNEL = make()


@jax.jit
def pallas_standalone__conformer_family_branchformer__speech_kernel(
    x: jax.Array,
    w_q: jax.Array,
    w_k: jax.Array,
    w_v: jax.Array,
    w_ao: jax.Array,
    w_up: jax.Array,
    dw: jax.Array,
    w_dn: jax.Array,
    w_merge: jax.Array,
):
    return _KERNEL(x, w_q, w_k, w_v, w_ao, w_up, dw, w_dn, w_merge)
```

```python
import functools
import math

import jax
import jax.numpy as jnp
import numpy as np
from jax import lax
import jax.experimental.pallas as pl
import jax.experimental.pallas.tpu as pltpu

F32 = jnp.float32
BF16 = jnp.bfloat16
EPS = 1e-5
LOG2E = 1.4426950408889634
HALO = 16
LN = 128


def _ln(x):
    m = jnp.mean(x, axis=-1, keepdims=True)
    xc = x - m
    v = jnp.mean(xc * xc, axis=-1, keepdims=True)
    return xc * lax.rsqrt(v + EPS)


def _gelu(x):
    c = math.sqrt(2.0 / math.pi)
    return (0.5 * x) * (1.0 + jnp.tanh(x * (c + (c * 0.044715) * (x * x))))


def _dot(a, b):
    return jnp.dot(a, b, preferred_element_type=F32)


def _dot_nt(a, b):
    return lax.dot_general(a, b, (((1,), (1,)), ((), ())), preferred_element_type=F32)


def _cat(xs):
    return jnp.concatenate(xs, axis=1)


def _spread(o, n):
    g = o.shape[0] // 8
    k = n // 8
    return jnp.concatenate([o[8 * (i * g // k):8 * (i * g // k) + 8] for i in range(k)], axis=0)


def _split(n, parts, p, unit=8):
    g = n // unit
    return unit * (p * g // parts), unit * ((p + 1) * g // parts)


def make(TQ=800, LNT=4, NEXP=6, flags=None):
    KC = 512
    HQ = TQ // 2
    HK = KC // 2

    def kernel(x_ref, wq_ref, wk_ref, wv_ref, wao_ref, wup_ref, dw_ref, wdn_ref, wm_ref,
               o_ref,
               wqk_s, wout_s, xa_s, y_s, dwb_s, z_s,
               g_s, cv_s, qf_s, q_s, h_s, m_s, r_s, l_s, ya_s, yc_s, o_s, s_s, p_s, acc_s,
               *, T, D, K, TP):
        b = pl.program_id(0)
        i = pl.program_id(1)
        NCH = TP // KC
        ND = D // LN
        lt = lambda c: slice(c * LN, (c + 1) * LN)
        top, bot = slice(0, HQ), slice(HQ, TQ)

        @pl.when((b == 0) & (i == 0))
        def _():
            scale = float(D) ** -0.5 * LOG2E

            def fold(c, carry):
                cs = pl.ds(pl.multiple_of(c * LN, LN), LN)
                wqk_s[:, cs] = (_dot_nt(wq_ref[...], wk_ref[cs, :]) * scale).astype(BF16)
                t = _dot(wao_ref[...], wm_ref[0:D, cs]).astype(BF16)
                wout_s[D:2 * D, cs] = _dot(wdn_ref[...], wm_ref[D:2 * D, cs]).astype(BF16)
                wout_s[0:D, cs] = _dot(wv_ref[...], t).astype(BF16)
                return carry
            lax.fori_loop(0, ND, fold, 0)
            z_s[0] = 0
            dw = dw_ref[...].astype(F32)
            for k in range(K):
                dwb_s[k] = jnp.broadcast_to(dw[k:k + 1, :], (8, D))
            for ref in (g_s, cv_s, qf_s, q_s, h_s, m_s, r_s, l_s, ya_s, yc_s, o_s, s_s, p_s, acc_s):
                ref[b, 0:16, :] = jnp.zeros((16, LN), ref.dtype)

        @pl.when(i == 0)
        def _():
            def chunk(j, rows):
                r0 = pl.multiple_of(j * KC, KC)
                xa = _ln(x_ref[pl.ds(r0, rows), :].astype(F32))
                if rows < KC:
                    xa = jnp.concatenate([xa, jnp.zeros((KC - rows, D), F32)], axis=0)
                for c in range(ND):
                    xa_s[c, pl.ds(r0, KC), :] = xa[:, lt(c)].astype(BF16)
                h0 = pl.multiple_of(j * HK, HK)
                for c in range(2):
                    x11, x12 = xa[0:HK, lt(c)], xa[0:HK, lt(2 + c)]
                    x21, x22 = xa[HK:KC, lt(c)], xa[HK:KC, lt(2 + c)]
                    ys = (x11 + x22, x11, x21 - x22, x12 - x11, x22, x11 + x21, x12 + x22)
                    for n, y in enumerate(ys):
                        y_s[2 * n + c, pl.ds(h0, HK), :] = y.astype(BF16)

            def body(j, carry):
                chunk(j, KC)
                return carry
            lax.fori_loop(0, T // KC, body, 0)
            if T % KC:
                chunk(T // KC, T % KC)
            x0 = _cat([xa_s[c, 0:HALO, :] for c in range(ND)])
            g0 = _ln(_gelu(_dot(x0, wup_ref[:, D:2 * D])))
            for c in range(ND):
                g_s[c, TQ:TQ + HALO, :] = jnp.zeros((HALO, LN), F32)
                g_s[c, TQ + HALO:TQ + 2 * HALO, :] = g0[:, lt(c)]

        r0 = pl.multiple_of(i * TQ, 16)
        never = lax.broadcasted_iota(jnp.int32, (8, LN), 1) < z_s[0]

        def after(v, o):
            n = v.shape[0]
            if o.shape[0] != n:
                o = _spread(o, n)
            return jnp.where(never[None], o.reshape(n // 8, 8, LN), v.reshape(n // 8, 8, LN)).reshape(n, LN)

        xrows = lambda r: _cat([xa_s[c, pl.ds(r, TQ), :] for c in range(ND)])
        pair = lambda ref, n: _cat([ref[2 * n], ref[2 * n + 1]])
        ykeys = lambda n, j: _cat([y_s[2 * n + c, j * HK:(j + 1) * HK, :] for c in range(2)])

        for c in (0, 2, 1, 3):
            qc = _dot(xrows(r0), wqk_s[:, lt(c)])
            if c == 0:
                qc = after(qc, jnp.zeros_like(qc))
            g_s[c, 0:2 * HALO, :] = after(g_s[c, TQ:TQ + 2 * HALO, :], qc)
            if c < 2:
                qf_s[c] = qc
            else:
                a11, a21 = qf_s[c - 2, top, :], qf_s[c - 2, bot, :]
                a12, a22 = qc[top], qc[bot]
                qs = (a11 + a22, a21 + a22, a11, a22, a11 + a12, a21 - a11, a12 - a22)
                for n, a in enumerate(qs):
                    q_s[2 * n + c - 2] = a.astype(BF16)

        for c in range(ND):
            h_s[c] = _gelu(_dot(xrows(r0 + HALO), wup_ref[:, lt(ND + c)]))

        def gate_norm(a0, a1, o):
            n = a1 - a0
            gg = _ln(_cat([h_s[c, a0:a1, :] for c in range(ND)]))
            for c in range(ND):
                gc = after(gg[:, lt(c)], o)
                if a1 == TQ:
                    row = lax.broadcasted_iota(jnp.int32, (HALO, LN), 0) + (r0 + TQ)
                    g_s[c, 2 * HALO + a0:HALO + TQ, :] = gc[0:n - HALO]
                    g_s[c, HALO + TQ:2 * HALO + TQ, :] = jnp.where(row < T, gc[n - HALO:n], 0.0)
                else:
                    g_s[c, 2 * HALO + a0:2 * HALO + a1, :] = gc

        def conv_part(c, a0, a1, o):
            rc = a1 - a0
            gt = g_s[c, a0:a1 + 2 * HALO, :].reshape((rc + 2 * HALO) // 8, 8, LN)
            acc = None
            for bb in range(8):
                n = rc // 8 + (1 if bb else 0)
                y = None
                for a in range(4):
                    k = 8 * a + bb - 1
                    if k < 0:
                        continue
                    t = gt[a:a + n] * dwb_s[k, :, lt(c)][None]
                    y = t if y is None else y + t
                y = y.reshape(n * 8, LN)[bb:bb + rc]
                acc = y if acc is None else acc + y
            cv_s[c, a0:a1, :] = after(acc, o)

        def local_branch(c):
            u = _gelu(_dot(xrows(r0), wup_ref[:, lt(c)]))
            yc_s[c] = (u * cv_s[c]).astype(BF16)
            o = _dot(yc_s[c], wout_s[D + c * LN:D + (c + 1) * LN, :])
            for n in range(ND):
                base = x_ref[pl.ds(r0, TQ), lt(n)].astype(F32) if c == 0 else o_s[n]
                o_s[n] = o[:, lt(n)] + base

        def finish(half, kt, s):
            if (kt + 1) * LN > T:
                col = lax.broadcasted_iota(jnp.int32, s.shape, 1) + kt * LN
                s = jnp.where(col < T, s, -jnp.inf)
            s_s[kt, half, :] = s
            return s

        def track(half, s0, s1, first):
            mx = jnp.maximum(s0, s1)
            m_s[0, half, :] = mx if first else jnp.maximum(mx, m_s[0, half, :])

        per = 7 * NCH // ND
        for j in range(NCH):
            ka, kb = 4 * j, 4 * j + 2
            for n in range(7):
                mm = _dot_nt(pair(q_s, n), ykeys(n, j))
                fin = []
                for c in range(2):
                    v = mm[:, lt(c)]
                    if n == 0:
                        s_s[ka + c, top, :] = v
                    elif n == 1:
                        s_s[kb + c, bot, :] = s_s[ka + c, top, :] - v
                        s_s[ka + c, bot, :] = v
                    elif n == 2:
                        s_s[kb + c, bot, :] = s_s[kb + c, bot, :] + v
                        s_s[kb + c, top, :] = v
                    elif n == 3:
                        s_s[ka + c, top, :] = s_s[ka + c, top, :] + v
                        fin.append(finish(bot, ka + c, s_s[ka + c, bot, :] + v))
                    elif n == 4:
                        s_s[ka + c, top, :] = s_s[ka + c, top, :] - v
                        fin.append(finish(top, kb + c, s_s[kb + c, top, :] + v))
                    elif n == 5:
                        fin.append(finish(bot, kb + c, s_s[kb + c, bot, :] + v))
                    else:
                        fin.append(finish(top, ka + c, s_s[ka + c, top, :] + v))
                if fin:
                    track(bot if n in (3, 5) else top, fin[0], fin[1], j == 0 and n < 5)
                t = 7 * j + n
                if t < LNT:
                    gate_norm(*_split(TQ, LNT, t), mm[:, lt(0)])
                else:
                    c, first = t // per, max(LNT, t // per * per)
                    conv_part(c, *_split(TQ, (c + 1) * per - first, t - first), mm[:, lt(0)])
                if (t + 1) % per == 0:
                    local_branch(t // per)

        lane_max = m_s[0]
        m = jnp.broadcast_to(jnp.max(lane_max, axis=-1, keepdims=True), (TQ, LN))
        est = jnp.sum(jnp.exp2(lane_max - m), axis=-1, keepdims=True)
        m_s[0] = m
        r_s[0] = jnp.broadcast_to(1.0 / est, (TQ, LN))

        def exp_rows(j, a0, a1, o):
            ka, kb = 4 * j, 4 * j + 2
            rt, rb = slice(a0, a1), slice(HQ + a0, HQ + a1)
            mt, mb, st, sb = m_s[0, rt, :], m_s[0, rb, :], r_s[0, rt, :], r_s[0, rb, :]
            lt_, lb_ = None, None
            for c in range(2):
                p11 = jnp.exp2(s_s[ka + c, rt, :] - mt) * st
                p12 = jnp.exp2(s_s[kb + c, rt, :] - mt) * st
                p21 = jnp.exp2(s_s[ka + c, rb, :] - mb) * sb
                p22 = jnp.exp2(s_s[kb + c, rb, :] - mb) * sb
                if o is not None:
                    p11, p22 = after(p11, o[:, lt(c)]), after(p22, o[:, lt(c)])
                ps = (p11 + p22, p21 - p22, p12 + p22, p11 + p21, p12 - p11, p22, p11)
                for n, p in enumerate(ps):
                    p_s[14 * (j % 2) + 2 * n + c, rt, :] = p.astype(BF16)
                lt_ = p11 + p12 if c == 0 else lt_ + (p11 + p12)
                lb_ = p21 + p22 if c == 0 else lb_ + (p21 + p22)
            if j > 0:
                lt_, lb_ = lt_ + l_s[0, rt, :], lb_ + l_s[0, rb, :]
            if j + 1 == NCH:
                lt_, lb_ = [jnp.broadcast_to(1.0 / jnp.sum(v, axis=-1, keepdims=True), v.shape) for v in (lt_, lb_)]
            l_s[0, rt, :] = lt_
            l_s[0, rb, :] = lb_

        N1, N3, N7, N6, N4, N5, N2 = range(7)
        order = (N1, N2, N4, N5, N7, N3, N6)
        exp_rows(0, 0, HQ, None)
        for j in range(NCH):
            for pos, n in enumerate(order):
                o = _dot(pair(p_s, 7 * (j % 2) + n), ykeys(n, j))
                if j + 1 < NCH and pos < NEXP:
                    exp_rows(j + 1, *_split(HQ, NEXP, pos, 16), o)
                for c in range(2):
                    v = o[:, lt(c)]
                    if j > 0:
                        v = v + acc_s[2 * n + c]
                    a = lambda k: acc_s[2 * k + c]
                    if j + 1 < NCH or n in (N1, N2, N3, N4, N5):
                        acc_s[2 * n + c] = v
                    if j + 1 == NCH:
                        if n == N4:
                            ya_s[2 + c, top, :] = ((a(N2) + v) * l_s[0, top, :]).astype(BF16)
                        elif n == N7:
                            ya_s[c, top, :] = (((a(N1) + a(N4)) + (v - a(N5))) * l_s[0, top, :]).astype(BF16)
                        elif n == N3:
                            ya_s[c, bot, :] = ((a(N5) + v) * l_s[0, bot, :]).astype(BF16)
                        elif n == N6:
                            ya_s[2 + c, bot, :] = (((a(N1) - a(N2)) + (a(N3) + v)) * l_s[0, bot, :]).astype(BF16)
        for c in range(ND):
            ya = _cat([ya_s[d] for d in range(ND)])
            o_ref[:, lt(c)] = (_dot(ya, wout_s[0:D, lt(c)]) + o_s[c]).astype(o_ref.dtype)

    @jax.jit
    def fn(x, w_q, w_k, w_v, w_ao, w_up, dw, w_dn, w_merge):
        B, T, D = x.shape
        K = dw.shape[0]
        TP = (T + KC - 1) // KC * KC
        NKT = TP // LN
        ND = D // LN
        full = lambda a: pl.BlockSpec(a.shape, lambda b, i: (0,) * a.ndim)
        V = pltpu.VMEM
        return pl.pallas_call(
            functools.partial(kernel, T=T, D=D, K=K, TP=TP),
            grid=(B, T // TQ),
            in_specs=[pl.BlockSpec((None, T, D), lambda b, i: (b, 0, 0))]
            + [full(a) for a in (w_q, w_k, w_v, w_ao, w_up, dw, w_dn, w_merge)],
            out_specs=pl.BlockSpec((None, TQ, D), lambda b, i: (b, i, 0)),
            out_shape=jax.ShapeDtypeStruct(x.shape, x.dtype),
            scratch_shapes=[
                V((D, D), BF16),
                V((2 * D, D), BF16),
                V((ND, TP, LN), BF16),
                V((14, TP // 2, LN), BF16),
                V((K, 8, D), F32),
                pltpu.SMEM((1,), jnp.int32),
                V((ND, TQ + 2 * HALO, LN), F32),
                V((ND, TQ, LN), F32),
                V((2, TQ, LN), F32),
                V((14, HQ, LN), BF16),
                V((ND, TQ, LN), F32),
                V((1, TQ, LN), F32),
                V((1, TQ, LN), F32),
                V((1, TQ, LN), F32),
                V((ND, TQ, LN), BF16),
                V((ND, TQ, LN), BF16),
                V((ND, TQ, LN), F32),
                V((NKT, TQ, LN), F32),
                V((28, HQ, LN), BF16),
                V((14, HQ, LN), F32),
            ],
            compiler_params=pltpu.CompilerParams(
                dimension_semantics=("arbitrary", "arbitrary"),
                vmem_limit_bytes=100 * 1024 * 1024,
                flags=flags,
            ),
        )(x, w_q, w_k, w_v, w_ao, w_up, dw, w_dn, w_merge)

    return fn


_KERNEL = make()


@jax.jit
def pallas_standalone__conformer_family_branchformer__speech_kernel(
    x: jax.Array,
    w_q: jax.Array,
    w_k: jax.Array,
    w_v: jax.Array,
    w_ao: jax.Array,
    w_up: jax.Array,
    dw: jax.Array,
    w_dn: jax.Array,
    w_merge: jax.Array,
):
    return _KERNEL(x, w_q, w_k, w_v, w_ao, w_up, dw, w_dn, w_merge)
```

```python
import functools
import math

import jax
import jax.numpy as jnp
import numpy as np
from jax import lax
import jax.experimental.pallas as pl
import jax.experimental.pallas.tpu as pltpu

F32 = jnp.float32
BF16 = jnp.bfloat16
EPS = 1e-5
LOG2E = 1.4426950408889634
HALO = 16
LN = 128


def _ln(x):
    m = jnp.mean(x, axis=-1, keepdims=True)
    xc = x - m
    v = jnp.mean(xc * xc, axis=-1, keepdims=True)
    return xc * lax.rsqrt(v + EPS)


def _gelu(x):
    c = math.sqrt(2.0 / math.pi)
    return (0.5 * x) * (1.0 + jnp.tanh(x * (c + (c * 0.044715) * (x * x))))


def _dot(a, b):
    return jnp.dot(a, b, preferred_element_type=F32)


def _dot_nt(a, b):
    return lax.dot_general(a, b, (((1,), (1,)), ((), ())), preferred_element_type=F32)


def _cat(xs):
    return jnp.concatenate(xs, axis=1)


def _spread(o, n):
    g = o.shape[0] // 8
    k = n // 8
    return jnp.concatenate([o[8 * (i * g // k):8 * (i * g // k) + 8] for i in range(k)], axis=0)


def _split(n, parts, p, unit=8):
    g = n // unit
    return unit * (p * g // parts), unit * ((p + 1) * g // parts)


def _left(a11, a12, a21, a22):
    return (a11 + a22, a21 + a22, a11, a22, a11 + a12, a21 - a11, a12 - a22)


def _right(b11, b12, b21, b22):
    return (b11 + b22, b11, b12 - b22, b21 - b11, b22, b11 + b12, b21 + b22)


SIGNS = {(0, 0): {0: 1, 3: 1, 4: -1, 6: 1}, (0, 1): {2: 1, 4: 1},
         (1, 0): {1: 1, 3: 1}, (1, 1): {0: 1, 1: -1, 2: 1, 5: 1}}


def _collect(order, n, v, load, store, done, opened=False):
    seen = order[:order.index(n)]
    for blk, signs in SIGNS.items():
        if n not in signs:
            continue
        if opened or any(k in signs for k in seen):
            t = load(blk) + v if signs[n] > 0 else load(blk) - v
        else:
            t = v if signs[n] > 0 else -v
        if all(k == n or k in seen for k in signs):
            done(blk, t)
        else:
            store(blk, t)


def make(HQ=400, LNT=4, NEXP=6, flags=None):
    TQ = 2 * HQ
    HK = 256

    def kernel(x_hbm, wq_hbm, wk_hbm, wv_hbm, wao_hbm, wup_hbm, dw_hbm, wdn_hbm, wm_hbm,
               o_ref,
               x_s, w_s, dw_ref, wsem, xsem,
               wf_s, wc_s, y_s, dwb_s, gb_s, z_s,
               g_s, cv_s, t_s, q_s, h_s, m_s, r_s, l_s, ya_s, yc_s, o_s, s_s, p_s, acc_s,
               *, T, D, K, HP):
        b = pl.program_id(0)
        i = pl.program_id(1)
        HT = T // 2
        HD = D // 2
        NCH = HP // HK
        ND = D // LN
        lt = lambda c: slice(c * LN, (c + 1) * LN)
        rows = (slice(0, HQ), slice(HQ, TQ))

        WAO, WV, WMA, TMP = 0, 1, 3, 4
        WDN, WMC, WQ, WK, WU, WG = 2, 6, 8, 9, 10, 11
        w_dma = [pltpu.make_async_copy(src, dst, wsem.at[n]) for n, (src, dst) in enumerate((
            (wq_hbm, w_s.at[WQ]), (wk_hbm, w_s.at[WK]), (wao_hbm, w_s.at[WAO]), (wm_hbm.at[0:D], w_s.at[WMA]),
            (wv_hbm, w_s.at[WV]), (wdn_hbm, w_s.at[WDN]), (wm_hbm.at[D:2 * D], w_s.at[WMC]),
            (dw_hbm, dw_ref), (wup_hbm.at[:, 0:D], w_s.at[WU]), (wup_hbm.at[:, D:2 * D], w_s.at[WG])))]
        F_VO, F_DC, F_QK, F_U, F_G = range(5)

        def x_dma(bb, half, j, n):
            return pltpu.make_async_copy(
                x_hbm.at[bb, pl.ds(pl.multiple_of(half * HT + j * HK, 16), n)],
                x_s.at[bb, half, pl.ds(pl.multiple_of(j * HK, HK), n)], xsem.at[half, j])

        def x_start(bb, j0, j1):
            for j in range(j0, j1):
                for half in range(2):
                    x_dma(bb, half, j, min(HK, HT - j * HK)).start()

        @pl.when((b == 0) & (i == 0))
        def _():
            for n in range(4):
                w_dma[n].start()
            for bb in range(x_s.shape[0]):
                for half in range(2):
                    x_s[bb, half, HT:HP, :] = jnp.zeros((HP - HT, D), BF16)
            cols = lambda c: pl.ds(pl.multiple_of(c * LN, LN), LN)
            w_dma[0].wait()
            w_dma[1].wait()
            for n in range(4, 7):
                w_dma[n].start()

            def fold_qk(c, carry):
                wf_s[F_QK, :, cols(c)] = _dot_nt(w_s[WQ], w_s[WK, cols(c), :]) * (float(D) ** -0.5 * LOG2E)
                return carry
            lax.fori_loop(0, ND, fold_qk, 0)
            w_dma[2].wait()
            w_dma[3].wait()
            x_start(0, 0, NCH // 2)

            def fold(t, carry):
                f, c = t // ND, t % ND

                @pl.when(t == ND)
                def _():
                    for n in range(4, 7):
                        w_dma[n].wait()
                    x_start(0, NCH // 2, NCH)
                    for n in range(7, 10):
                        w_dma[n].start()

                rhs = jnp.where(f == 2, WMC, WMA + f)
                v = _dot(w_s[f], w_s[rhs, :, cols(c)])
                w_s[rhs + 1, :, cols(c)] = v.astype(BF16)
                wf_s[jnp.maximum(f - 1, 0), :, cols(c)] = v
                return carry
            lax.fori_loop(0, 3 * ND, fold, 0)
            z_s[0] = 0
            for ref in (g_s, cv_s, t_s, q_s, h_s, m_s, r_s, l_s, ya_s, yc_s, o_s, s_s, p_s, acc_s):
                ref[b, 0:16, :] = jnp.zeros((16, LN), ref.dtype)

        @pl.when(i == 0)
        def _():
            def chunk(j, carry):
                h0 = pl.multiple_of(j * HK, HK)

                @pl.when(j < HT // HK)
                def _():
                    for half in range(2):
                        x_dma(b, half, j, HK).wait()

                if HT % HK:
                    @pl.when(j == HT // HK)
                    def _():
                        for half in range(2):
                            x_dma(b, half, j, HT % HK).wait()

                xa, xb = [_ln(x_s[b, half, pl.ds(h0, HK), :].astype(F32)) for half in range(2)]
                for c in range(2):
                    ys = _right(xa[:, lt(c)], xb[:, lt(c)], xa[:, lt(2 + c)], xb[:, lt(2 + c)])
                    for n, y in enumerate(ys):
                        y_s[2 * n + c, pl.ds(h0, HK), :] = y.astype(BF16)
                return carry
            lax.fori_loop(0, NCH, chunk, 0)

            @pl.when(b == 0)
            def _():
                for n in range(7, 10):
                    w_dma[n].wait()
                dw = dw_ref[...].astype(F32)
                for k in range(K):
                    dwb_s[k] = jnp.broadcast_to(dw[k:k + 1, :], (8, D))

                def blocks(f):
                    return (wf_s[f, 0:HD, 0:HD], wf_s[f, 0:HD, HD:D], wf_s[f, HD:D, 0:HD], wf_s[f, HD:D, HD:D])

                def right(f, carry):
                    for n, w in enumerate(_right(*blocks(f))):
                        wc_s[f, n] = w.astype(BF16)
                    return carry
                lax.fori_loop(F_VO, F_QK, right, 0)

                def left(f, carry):
                    @pl.when(f > F_QK)
                    def _():
                        wf_s[f] = w_s[WU + f - F_U].astype(F32)
                    w11, w12, w21, w22 = blocks(f)
                    for n, w in enumerate(_left(w11, w21, w12, w22)):
                        wc_s[f, n] = w.astype(BF16)
                    return carry
                lax.fori_loop(F_QK, F_G + 1, left, 0)

            @pl.when(b + 1 < pl.num_programs(0))
            def _():
                x_start(b + 1, 0, NCH)

            x0 = jnp.concatenate([x_s[b, 0, 0:HALO, :], x_s[b, 0, HT - HALO:HT, :], x_s[b, 1, 0:HALO, :]], axis=0)
            g0 = _ln(_gelu(_dot(_ln(x0.astype(F32)).astype(BF16), w_s[WG])))
            gb_s[...] = g0[2 * HALO:3 * HALO]
            for c in range(ND):
                g_s[c, HQ:HQ + HALO, :] = jnp.zeros((HALO, LN), F32)
                g_s[c, HQ + HALO:HQ + 2 * HALO, :] = g0[0:HALO, lt(c)]
                g_s[ND + c, HQ:HQ + 2 * HALO, :] = g0[HALO:3 * HALO, lt(c)]

        h0 = pl.multiple_of(i * HQ, 16)
        never = lax.broadcasted_iota(jnp.int32, (8, LN), 1) < z_s[0]

        def after(v, o):
            n = v.shape[0]
            if o.shape[0] != n:
                o = _spread(o, n)
            return jnp.where(never[None], o.reshape(n // 8, 8, LN), v.reshape(n // 8, 8, LN)).reshape(n, LN)

        pair = lambda ref, n: _cat([ref[2 * n], ref[2 * n + 1]])
        ykeys = lambda n, j: _cat([y_s[2 * n + c, j * HK:(j + 1) * HK, :] for c in range(2)])

        def project(f, r, ref, done, hook=None):
            order = (1, 3, 2, 4, 0, 5, 6)
            for n in order:
                mm = _dot(_cat([y_s[2 * n + c, pl.ds(r, HQ), :] for c in range(2)]), wc_s[f, n])
                for c in range(2):
                    def store(blk, t):
                        ref[2 * blk[0] + c, rows[blk[1]], :] = t
                    _collect(order, n, mm[:, lt(c)], lambda blk: ref[2 * blk[0] + c, rows[blk[1]], :], store,
                             lambda blk, t: done(2 * blk[0] + c, blk[1], t))
                if hook is not None:
                    hook(order.index(n), mm[:, lt(0)])

        def operands(dst):
            def done(c, half, t):
                if (c // 2, half) != (0, 0):
                    t_s[c, rows[half], :] = t
                else:
                    blocks = (t, t_s[c + 2, rows[0], :], t_s[c, rows[1], :], t_s[c + 2, rows[1], :])
                    for n, a in enumerate(_left(*blocks)):
                        dst[2 * n + c] = a.astype(BF16)
            return done

        def carry_halo(pos, o):
            if pos < ND:
                for k in (pos, ND + pos):
                    g_s[k, 0:2 * HALO, :] = after(g_s[k, HQ:HQ + 2 * HALO, :], o)

        project(F_QK, h0, t_s, operands(q_s), carry_halo)

        def gate_done(c, half, t):
            h_s[c, rows[half], :] = _gelu(t)
        project(F_G, h0 + HALO, h_s, gate_done)

        def gate_norm(half, a0, a1, o):
            n = a1 - a0
            gg = _ln(_cat([h_s[c, half * HQ + a0:half * HQ + a1, :] for c in range(ND)]))
            for c in range(ND):
                gc = after(gg[:, lt(c)], o)
                k = half * ND + c
                if a1 == HQ:
                    row = lax.broadcasted_iota(jnp.int32, (HALO, LN), 0) + (h0 + HQ)
                    past = gb_s[:, lt(c)] if half == 0 else 0.0
                    g_s[k, 2 * HALO + a0:HALO + HQ, :] = gc[0:n - HALO]
                    g_s[k, HALO + HQ:2 * HALO + HQ, :] = jnp.where(row < HT, gc[n - HALO:n], past)
                else:
                    g_s[k, 2 * HALO + a0:2 * HALO + a1, :] = gc

        def conv_part(half, c, a0, a1, o):
            rc = a1 - a0
            gt = g_s[half * ND + c, a0:a1 + 2 * HALO, :].reshape((rc + 2 * HALO) // 8, 8, LN)
            acc = None
            for bb in range(8):
                n = rc // 8 + (1 if bb else 0)
                y = None
                for a in range(4):
                    k = 8 * a + bb - 1
                    if k < 0:
                        continue
                    t = gt[a:a + n] * dwb_s[k, :, lt(c)][None]
                    y = t if y is None else y + t
                y = y.reshape(n * 8, LN)[bb:bb + rc]
                acc = y if acc is None else acc + y
            cv_s[c, half * HQ + a0:half * HQ + a1, :] = after(acc, o)

        def unproject(f, src, order, first, done):
            for n in order:
                mm = _dot(pair(src, n), wc_s[f, n])
                for c in range(2):
                    seen = order[:order.index(n)]

                    def load(blk):
                        cc = 2 * blk[1] + c
                        if first and not any(k in SIGNS[blk] for k in seen):
                            return x_s[b, blk[0], pl.ds(h0, HQ), lt(cc)].astype(F32)
                        return o_s[cc, rows[blk[0]], :]

                    def store(blk, t):
                        o_s[2 * blk[1] + c, rows[blk[0]], :] = t
                    _collect(order, n, mm[:, lt(c)], load, store,
                             (lambda blk, t: done(2 * blk[1] + c, blk[0], t)) if done else store, opened=True)

        nslots = 7 * (NCH - 1) - LNT
        per = nslots // (2 * ND)
        order = tuple(range(7))
        for j in range(NCH):
            if j == NCH - 1:
                local = operands(yc_s)
                project(F_U, h0, t_s, lambda c, half, t: local(c, half, _gelu(t) * cv_s[c, rows[half], :]))
            for n in order:
                mm = _dot_nt(pair(q_s, n), ykeys(n, j))
                fin = []
                for c in range(2):
                    def store(blk, t):
                        s_s[4 * j + 2 * blk[1] + c, rows[blk[0]], :] = t

                    def done(blk, t):
                        k0 = j * HK + c * LN
                        if k0 + LN > HT:
                            col = lax.broadcasted_iota(jnp.int32, t.shape, 1) + k0
                            t = jnp.where(col < HT, t, -jnp.inf)
                        store(blk, t)
                        fin.append((blk, t))
                    _collect(order, n, mm[:, lt(c)], lambda blk: s_s[4 * j + 2 * blk[1] + c, rows[blk[0]], :], store, done)
                if fin:
                    rr = rows[fin[0][0][0]]
                    mx = jnp.maximum(fin[0][1], fin[1][1])
                    m_s[0, rr, :] = mx if (j == 0 and n < 5) else jnp.maximum(mx, m_s[0, rr, :])
                t = 7 * j + n
                if t < LNT:
                    gate_norm(t % 2, *_split(HQ, LNT // 2, t // 2), mm[:, lt(0)])
                elif t - LNT < per * 2 * ND:
                    k = (t - LNT) // per
                    conv_part(k % 2, k // 2, *_split(HQ, per, (t - LNT) % per), mm[:, lt(0)])

        unproject(F_DC, yc_s, order, True, None)

        lane_max = m_s[0]
        m = jnp.broadcast_to(jnp.max(lane_max, axis=-1, keepdims=True), (TQ, LN))
        est = jnp.sum(jnp.exp2(lane_max - m), axis=-1, keepdims=True)
        m_s[0] = m
        r_s[0] = jnp.broadcast_to(1.0 / est, (TQ, LN))

        def exp_rows(j, a0, a1, o):
            ka, kb = 4 * j, 4 * j + 2
            rt, rb = slice(a0, a1), slice(HQ + a0, HQ + a1)
            mt, mb, st, sb = m_s[0, rt, :], m_s[0, rb, :], r_s[0, rt, :], r_s[0, rb, :]
            lt_, lb_ = None, None
            for c in range(2):
                p11 = jnp.exp2(s_s[ka + c, rt, :] - mt) * st
                p12 = jnp.exp2(s_s[kb + c, rt, :] - mt) * st
                p21 = jnp.exp2(s_s[ka + c, rb, :] - mb) * sb
                p22 = jnp.exp2(s_s[kb + c, rb, :] - mb) * sb
                if o is not None:
                    p11, p22 = after(p11, o[:, lt(c)]), after(p22, o[:, lt(c)])
                for n, p in enumerate(_right(p11, p21, p12, p22)):
                    p_s[14 * (j % 2) + 2 * n + c, rt, :] = p.astype(BF16)
                lt_ = p11 + p12 if c == 0 else lt_ + (p11 + p12)
                lb_ = p21 + p22 if c == 0 else lb_ + (p21 + p22)
            if j > 0:
                lt_, lb_ = lt_ + l_s[0, rt, :], lb_ + l_s[0, rb, :]
            if j + 1 == NCH:
                lt_, lb_ = [jnp.broadcast_to(1.0 / jnp.sum(v, axis=-1, keepdims=True), v.shape) for v in (lt_, lb_)]
            l_s[0, rt, :] = lt_
            l_s[0, rb, :] = lb_

        y_of = (0, 6, 1, 4, 5, 3, 2)
        order = (2, 4, 1, 3, 0, 5, 6)
        mixed = operands(ya_s)
        exp_rows(0, 0, HQ, None)
        for j in range(NCH):
            for pos, n in enumerate(order):
                o = _dot(pair(p_s, 7 * (j % 2) + n), ykeys(y_of[n], j))
                if j + 1 < NCH and pos < NEXP:
                    exp_rows(j + 1, *_split(HQ, NEXP, pos, 16), o)
                for c in range(2):
                    v = o[:, lt(c)]
                    if j > 0:
                        v = v + acc_s[2 * n + c]
                    if j + 1 < NCH or pos < 5:
                        acc_s[2 * n + c] = v
                    if j + 1 == NCH:
                        for blk, signs in SIGNS.items():
                            if n in signs and all(k in order[:pos + 1] for k in signs):
                                t = v
                                for k, sg in signs.items():
                                    if k != n:
                                        t = t + acc_s[2 * k + c] if sg > 0 else t - acc_s[2 * k + c]
                                mixed(2 * blk[0] + c, blk[1], t * l_s[0, rows[blk[1]], :])

        def out_done(c, half, t):
            o_ref[half, :, lt(c)] = t.astype(o_ref.dtype)
        unproject(F_VO, ya_s, (1, 3, 5, 2, 4, 0, 6), False, out_done)

    @jax.jit
    def fn(x, w_q, w_k, w_v, w_ao, w_up, dw, w_dn, w_merge):
        B, T, D = x.shape
        K = dw.shape[0]
        HT = T // 2
        HP = (HT + HK - 1) // HK * HK
        ND = D // LN
        V = pltpu.VMEM
        out = pl.pallas_call(
            functools.partial(kernel, T=T, D=D, K=K, HP=HP),
            grid=(B, HT // HQ),
            in_specs=[pl.BlockSpec(memory_space=pl.ANY)] * 9,
            out_specs=pl.BlockSpec((None, 2, HQ, D), lambda b, i: (b, 0, i, 0)),
            out_shape=jax.ShapeDtypeStruct((B, 2, HT, D), x.dtype),
            scratch_shapes=[
                V((B, 2, HP, D), BF16),
                V((12, D, D), BF16),
                V(dw.shape, BF16),
                pltpu.SemaphoreType.DMA((10,)),
                pltpu.SemaphoreType.DMA((2, HP // HK)),
                V((5, D, D), F32),
                V((5, 7, D // 2, D // 2), BF16),
                V((14, HP, LN), BF16),
                V((K, 8, D), F32),
                V((HALO, D), F32),
                pltpu.SMEM((1,), jnp.int32),
                V((2 * ND, HQ + 2 * HALO, LN), F32),
                V((ND, TQ, LN), F32),
                V((ND, TQ, LN), F32),
                V((14, HQ, LN), BF16),
                V((ND, TQ, LN), F32),
                V((1, TQ, LN), F32),
                V((1, TQ, LN), F32),
                V((1, TQ, LN), F32),
                V((14, HQ, LN), BF16),
                V((14, HQ, LN), BF16),
                V((ND, TQ, LN), F32),
                V((2 * HP // LN, TQ, LN), F32),
                V((28, HQ, LN), BF16),
                V((14, HQ, LN), F32),
            ],
            compiler_params=pltpu.CompilerParams(
                dimension_semantics=("arbitrary", "arbitrary"),
                vmem_limit_bytes=100 * 1024 * 1024,
                flags=flags,
            ),
        )(x, w_q, w_k, w_v, w_ao, w_up, dw, w_dn, w_merge)
        return out.reshape(B, T, D)

    return fn


_KERNEL = make()


@jax.jit
def pallas_standalone__conformer_family_branchformer__speech_kernel(
    x: jax.Array,
    w_q: jax.Array,
    w_k: jax.Array,
    w_v: jax.Array,
    w_ao: jax.Array,
    w_up: jax.Array,
    dw: jax.Array,
    w_dn: jax.Array,
    w_merge: jax.Array,
):
    return _KERNEL(x, w_q, w_k, w_v, w_ao, w_up, dw, w_dn, w_merge)
```

```python
import functools
import math

import jax
import jax.numpy as jnp
import numpy as np
from jax import lax
import jax.experimental.pallas as pl
import jax.experimental.pallas.tpu as pltpu

F32 = jnp.float32
BF16 = jnp.bfloat16
EPS = 1e-5
LOG2E = 1.4426950408889634
HALO = 16
LN = 128


def _ln(x):
    m = jnp.mean(x, axis=-1, keepdims=True)
    xc = x - m
    v = jnp.mean(xc * xc, axis=-1, keepdims=True)
    return xc * lax.rsqrt(v + EPS)


def _gelu(x):
    c = math.sqrt(2.0 / math.pi)
    return (0.5 * x) * (1.0 + jnp.tanh(x * (c + (c * 0.044715) * (x * x))))


def _dot(a, b):
    return jnp.dot(a, b, preferred_element_type=F32)


def _dot_nt(a, b):
    return lax.dot_general(a, b, (((1,), (1,)), ((), ())), preferred_element_type=F32)


def _cat(xs):
    return jnp.concatenate(xs, axis=1)


def _spread(o, n):
    g = o.shape[0] // 8
    k = n // 8
    return jnp.concatenate([o[8 * (i * g // k):8 * (i * g // k) + 8] for i in range(k)], axis=0)


def _split(n, parts, p, unit=8):
    g = n // unit
    return unit * (p * g // parts), unit * ((p + 1) * g // parts)


def _left(a11, a12, a21, a22):
    return (a11 + a22, a21 + a22, a11, a22, a11 + a12, a21 - a11, a12 - a22)


def _right(b11, b12, b21, b22):
    return (b11 + b22, b11, b12 - b22, b21 - b11, b22, b11 + b12, b21 + b22)


SIGNS = {(0, 0): {0: 1, 3: 1, 4: -1, 6: 1}, (0, 1): {2: 1, 4: 1},
         (1, 0): {1: 1, 3: 1}, (1, 1): {0: 1, 1: -1, 2: 1, 5: 1}}


def _collect(order, n, v, load, store, done, opened=False):
    seen = order[:order.index(n)]
    for blk, signs in SIGNS.items():
        if n not in signs:
            continue
        if opened or any(k in signs for k in seen):
            t = load(blk) + v if signs[n] > 0 else load(blk) - v
        else:
            t = v if signs[n] > 0 else -v
        if all(k == n or k in seen for k in signs):
            done(blk, t)
        else:
            store(blk, t)


def make(HQ=400, LNT=4, NEXP=6, XA=2, FN=256, NX=6, NY=6, flags=None):
    TQ = 2 * HQ
    HK = 256

    def kernel(x_hbm, wq_hbm, wk_hbm, wv_hbm, wao_hbm, wup_hbm, dw_hbm, wdn_hbm, wm_hbm,
               o_ref,
               x_s, w_s, dw_ref, wsem, xsem,
               wf_s, wc_s, y_s, dwb_s, gb_s, z_s,
               g_s, cv_s, t_s, q_s, h_s, m_s, r_s, l_s, ya_s, yc_s, o_s, s_s, p_s, acc_s,
               *, T, D, K, HP):
        b = pl.program_id(0)
        i = pl.program_id(1)
        HT = T // 2
        HD = D // 2
        NCH = HP // HK
        ND = D // LN
        lt = lambda c: slice(c * LN, (c + 1) * LN)
        rows = (slice(0, HQ), slice(HQ, TQ))

        WAO, WV, WMA, TMP = 0, 1, 3, 4
        WDN, WMC, WQ, WK, WU, WG = 2, 6, 8, 9, 10, 11
        w_dma = [pltpu.make_async_copy(src, dst, wsem.at[n]) for n, (src, dst) in enumerate((
            (wq_hbm, w_s.at[WQ]), (wk_hbm, w_s.at[WK]), (wao_hbm, w_s.at[WAO]), (wm_hbm.at[0:D], w_s.at[WMA]),
            (wv_hbm, w_s.at[WV]), (wdn_hbm, w_s.at[WDN]), (wm_hbm.at[D:2 * D], w_s.at[WMC]),
            (dw_hbm, dw_ref), (wup_hbm.at[:, 0:D], w_s.at[WU]), (wup_hbm.at[:, D:2 * D], w_s.at[WG])))]
        F_VO, F_DC, F_QK, F_U, F_G = range(5)

        NB = x_s.shape[0]
        NI = HT // HQ

        def x_dma(bb, j):
            r = pl.ds(pl.multiple_of(j * HQ, 16), HQ)
            return pltpu.make_async_copy(x_hbm.at[bb, :, r], x_s.at[bb, :, r], xsem.at[j])

        def store_operands(slot, r, n, c, blocks):
            for k, y in enumerate(_right(*blocks)):
                y_s[14 * slot + 2 * k + c, pl.ds(r, n), :] = y.astype(BF16)

        @pl.when((b == 0) & (i == 0))
        def _():
            for n in range(4):
                w_dma[n].start()
            y_s[:, HT:HP, :] = jnp.zeros((y_s.shape[0], HP - HT, LN), BF16)
            cols = lambda c: pl.ds(pl.multiple_of(c * FN, FN), FN)
            w_dma[0].wait()
            w_dma[1].wait()
            for n in range(4, 7):
                w_dma[n].start()

            def fold_qk(c, carry):
                wf_s[F_QK, :, cols(c)] = _dot_nt(w_s[WQ], w_s[WK, cols(c), :]) * (float(D) ** -0.5 * LOG2E)
                return carry
            lax.fori_loop(0, D // FN, fold_qk, 0)
            w_dma[2].wait()
            w_dma[3].wait()
            for j in range(XA):
                x_dma(0, j).start()

            def fold(t, carry):
                f, c = t // (D // FN), t % (D // FN)

                @pl.when(t == D // FN)
                def _():
                    for n in range(4, 7):
                        w_dma[n].wait()
                    for j in range(XA, NI):
                        x_dma(0, j).start()
                    for n in range(7, 10):
                        w_dma[n].start()

                rhs = jnp.where(f == 2, WMC, WMA + f)
                v = _dot(w_s[f], w_s[rhs, :, cols(c)])
                w_s[rhs + 1, :, cols(c)] = v.astype(BF16)
                wf_s[jnp.maximum(f - 1, 0), :, cols(c)] = v
                return carry
            lax.fori_loop(0, 3 * D // FN, fold, 0)
            z_s[0] = 0
            for ref in (g_s, cv_s, t_s, q_s, h_s, m_s, r_s, l_s, ya_s, yc_s, o_s, s_s, p_s, acc_s):
                ref[b, 0:16, :] = jnp.zeros((16, LN), ref.dtype)

            def first(j, carry):
                x_dma(0, j).wait()
                r = pl.multiple_of(j * HQ, 16)
                xa, xb = [_ln(x_s[0, half, pl.ds(r, HQ), :].astype(F32)) for half in range(2)]
                for c in range(2):
                    store_operands(0, r, HQ, c, (xa[:, lt(c)], xb[:, lt(c)], xa[:, lt(2 + c)], xb[:, lt(2 + c)]))
                return carry
            lax.fori_loop(0, NI, first, 0)
            if NB > 1:
                x_dma(1, 0).start()

            if True:
                for n in range(7, 10):
                    w_dma[n].wait()
                dw = dw_ref[...].astype(F32)
                for k in range(K):
                    dwb_s[k] = jnp.broadcast_to(dw[k:k + 1, :], (8, D))

                def blocks(f):
                    return (wf_s[f, 0:HD, 0:HD], wf_s[f, 0:HD, HD:D], wf_s[f, HD:D, 0:HD], wf_s[f, HD:D, HD:D])

                def right(f, carry):
                    for n, w in enumerate(_right(*blocks(f))):
                        wc_s[f, n] = w.astype(BF16)
                    return carry
                lax.fori_loop(F_VO, F_QK, right, 0)

                def left(f, carry):
                    @pl.when(f > F_QK)
                    def _():
                        wf_s[f] = w_s[WU + f - F_U].astype(F32)
                    w11, w12, w21, w22 = blocks(f)
                    for n, w in enumerate(_left(w11, w21, w12, w22)):
                        wc_s[f, n] = w.astype(BF16)
                    return carry
                lax.fori_loop(F_QK, F_G + 1, left, 0)

        @pl.when(i == 0)
        def _():
            x0 = jnp.concatenate([x_s[b, 0, 0:HALO, :], x_s[b, 0, HT - HALO:HT, :], x_s[b, 1, 0:HALO, :]], axis=0)
            g0 = _ln(_gelu(_dot(_ln(x0.astype(F32)).astype(BF16), w_s[WG])))
            gb_s[...] = g0[2 * HALO:3 * HALO]
            for c in range(ND):
                g_s[c, HQ:HQ + HALO, :] = jnp.zeros((HALO, LN), F32)
                g_s[c, HQ + HALO:HQ + 2 * HALO, :] = g0[0:HALO, lt(c)]
                g_s[ND + c, HQ:HQ + 2 * HALO, :] = g0[HALO:3 * HALO, lt(c)]

        @pl.when(b + 1 < NB)
        def _():
            x_dma(b + 1, i).wait()

        nxt = b * NI + i + 1

        @pl.when(nxt // NI + 1 < NB)
        def _():
            x_dma(nxt // NI + 1, nxt % NI).start()

        h0 = pl.multiple_of(i * HQ, 16)
        ys = 14 * (b % 2)
        never = lax.broadcasted_iota(jnp.int32, (8, LN), 1) < z_s[0]

        def after(v, o):
            n = v.shape[0]
            if o.shape[0] != n:
                o = _spread(o, n)
            return jnp.where(never[None], o.reshape(n // 8, 8, LN), v.reshape(n // 8, 8, LN)).reshape(n, LN)

        pair = lambda ref, n: _cat([ref[2 * n], ref[2 * n + 1]])
        ykeys = lambda n, j: _cat([y_s[ys + 2 * n + c, j * HK:(j + 1) * HK, :] for c in range(2)])

        def project(f, r, ref, done, hook=None):
            order = (1, 3, 2, 4, 0, 5, 6)
            for n in order:
                mm = _dot(_cat([y_s[ys + 2 * n + c, pl.ds(r, HQ), :] for c in range(2)]), wc_s[f, n])
                for c in range(2):
                    def store(blk, t):
                        ref[2 * blk[0] + c, rows[blk[1]], :] = t
                    _collect(order, n, mm[:, lt(c)], lambda blk: ref[2 * blk[0] + c, rows[blk[1]], :], store,
                             lambda blk, t: done(2 * blk[0] + c, blk[1], t))
                if hook is not None:
                    hook(order.index(n), mm[:, lt(0)])

        def operands(dst):
            def done(c, half, t):
                if (c // 2, half) != (0, 0):
                    t_s[c, rows[half], :] = t
                else:
                    blocks = (t, t_s[c + 2, rows[0], :], t_s[c, rows[1], :], t_s[c + 2, rows[1], :])
                    for n, a in enumerate(_left(*blocks)):
                        dst[2 * n + c] = a.astype(BF16)
            return done

        def carry_halo(pos, o):
            if pos < ND:
                for k in (pos, ND + pos):
                    g_s[k, 0:2 * HALO, :] = after(g_s[k, HQ:HQ + 2 * HALO, :], o)

        project(F_QK, h0, t_s, operands(q_s), carry_halo)

        def gate_done(c, half, t):
            h_s[c, rows[half], :] = _gelu(t)
        project(F_G, h0 + HALO, h_s, gate_done)

        def gate_norm(half, a0, a1, o):
            n = a1 - a0
            gg = _ln(_cat([h_s[c, half * HQ + a0:half * HQ + a1, :] for c in range(ND)]))
            for c in range(ND):
                gc = after(gg[:, lt(c)], o)
                k = half * ND + c
                if a1 == HQ:
                    row = lax.broadcasted_iota(jnp.int32, (HALO, LN), 0) + (h0 + HQ)
                    past = gb_s[:, lt(c)] if half == 0 else 0.0
                    g_s[k, 2 * HALO + a0:HALO + HQ, :] = gc[0:n - HALO]
                    g_s[k, HALO + HQ:2 * HALO + HQ, :] = jnp.where(row < HT, gc[n - HALO:n], past)
                else:
                    g_s[k, 2 * HALO + a0:2 * HALO + a1, :] = gc

        def conv_part(half, c, a0, a1, o):
            rc = a1 - a0
            gt = g_s[half * ND + c, a0:a1 + 2 * HALO, :].reshape((rc + 2 * HALO) // 8, 8, LN)
            acc = None
            for bb in range(8):
                n = rc // 8 + (1 if bb else 0)
                y = None
                for a in range(4):
                    k = 8 * a + bb - 1
                    if k < 0:
                        continue
                    t = gt[a:a + n] * dwb_s[k, :, lt(c)][None]
                    y = t if y is None else y + t
                y = y.reshape(n * 8, LN)[bb:bb + rc]
                acc = y if acc is None else acc + y
            cv_s[c, half * HQ + a0:half * HQ + a1, :] = after(acc, o)

        def unproject(f, src, order, first, done, results=None):
            for n in order:
                mm = _dot(pair(src, n), wc_s[f, n])
                if results is not None:
                    results.append(mm)
                for c in range(2):
                    seen = order[:order.index(n)]

                    def load(blk):
                        cc = 2 * blk[1] + c
                        if first and not any(k in SIGNS[blk] for k in seen):
                            return x_s[b, blk[0], pl.ds(h0, HQ), lt(cc)].astype(F32)
                        return o_s[cc, rows[blk[0]], :]

                    def store(blk, t):
                        o_s[2 * blk[1] + c, rows[blk[0]], :] = t
                    _collect(order, n, mm[:, lt(c)], load, store,
                             (lambda blk, t: done(2 * blk[1] + c, blk[0], t)) if done else store, opened=True)

        nslots = 7 * (NCH - 1) - LNT
        per = nslots // (2 * ND)
        order = tuple(range(7))
        for j in range(NCH):
            if j == NCH - 1:
                local = operands(yc_s)
                project(F_U, h0, t_s, lambda c, half, t: local(c, half, _gelu(t) * cv_s[c, rows[half], :]))
            for n in order:
                mm = _dot_nt(pair(q_s, n), ykeys(n, j))
                fin = []
                for c in range(2):
                    def store(blk, t):
                        s_s[4 * j + 2 * blk[1] + c, rows[blk[0]], :] = t

                    def done(blk, t):
                        k0 = j * HK + c * LN
                        if k0 + LN > HT:
                            col = lax.broadcasted_iota(jnp.int32, t.shape, 1) + k0
                            t = jnp.where(col < HT, t, -jnp.inf)
                        store(blk, t)
                        fin.append((blk, t))
                    _collect(order, n, mm[:, lt(c)], lambda blk: s_s[4 * j + 2 * blk[1] + c, rows[blk[0]], :], store, done)
                if fin:
                    rr = rows[fin[0][0][0]]
                    mx = jnp.maximum(fin[0][1], fin[1][1])
                    m_s[0, rr, :] = mx if (j == 0 and n < 5) else jnp.maximum(mx, m_s[0, rr, :])
                t = 7 * j + n
                if t < LNT:
                    gate_norm(t % 2, *_split(HQ, LNT // 2, t // 2), mm[:, lt(0)])
                elif t - LNT < per * 2 * ND:
                    k = (t - LNT) // per
                    conv_part(k % 2, k // 2, *_split(HQ, per, (t - LNT) % per), mm[:, lt(0)])

        unproject(F_DC, yc_s, order, True, None)

        lane_max = m_s[0]
        m = jnp.broadcast_to(jnp.max(lane_max, axis=-1, keepdims=True), (TQ, LN))
        est = jnp.sum(jnp.exp2(lane_max - m), axis=-1, keepdims=True)
        m_s[0] = m
        r_s[0] = jnp.broadcast_to(1.0 / est, (TQ, LN))

        def exp_rows(j, a0, a1, o):
            ka, kb = 4 * j, 4 * j + 2
            rt, rb = slice(a0, a1), slice(HQ + a0, HQ + a1)
            mt, mb, st, sb = m_s[0, rt, :], m_s[0, rb, :], r_s[0, rt, :], r_s[0, rb, :]
            lt_, lb_ = None, None
            for c in range(2):
                p11 = jnp.exp2(s_s[ka + c, rt, :] - mt) * st
                p12 = jnp.exp2(s_s[kb + c, rt, :] - mt) * st
                p21 = jnp.exp2(s_s[ka + c, rb, :] - mb) * sb
                p22 = jnp.exp2(s_s[kb + c, rb, :] - mb) * sb
                if o is not None:
                    p11, p22 = after(p11, o[:, lt(c)]), after(p22, o[:, lt(c)])
                for n, p in enumerate(_right(p11, p21, p12, p22)):
                    p_s[14 * (j % 2) + 2 * n + c, rt, :] = p.astype(BF16)
                lt_ = p11 + p12 if c == 0 else lt_ + (p11 + p12)
                lb_ = p21 + p22 if c == 0 else lb_ + (p21 + p22)
            if j > 0:
                lt_, lb_ = lt_ + l_s[0, rt, :], lb_ + l_s[0, rb, :]
            if j + 1 == NCH:
                lt_, lb_ = [jnp.broadcast_to(1.0 / jnp.sum(v, axis=-1, keepdims=True), v.shape) for v in (lt_, lb_)]
            l_s[0, rt, :] = lt_
            l_s[0, rb, :] = lb_

        y_of = (0, 6, 1, 4, 5, 3, 2)
        order = (2, 4, 1, 3, 0, 5, 6)
        mixed = operands(ya_s)
        exp_rows(0, 0, HQ, None)
        for j in range(NCH):
            for pos, n in enumerate(order):
                o = _dot(pair(p_s, 7 * (j % 2) + n), ykeys(y_of[n], j))
                if j + 1 < NCH and pos < NEXP:
                    exp_rows(j + 1, *_split(HQ, NEXP, pos, 16), o)
                if j + 1 == NCH and pos < NX:
                    a0, a1 = _split(HQ, NX, pos, 16)
                    for half in range(2):
                        xn = _ln(x_s[jnp.minimum(b + 1, NB - 1), half, pl.ds(h0 + a0, a1 - a0), :].astype(F32))
                        for c in range(ND):
                            h_s[c, half * HQ + a0:half * HQ + a1, :] = after(xn[:, lt(c)], o[:, lt(half)])
                for c in range(2):
                    v = o[:, lt(c)]
                    if j > 0:
                        v = v + acc_s[2 * n + c]
                    if j + 1 < NCH or pos < 5:
                        acc_s[2 * n + c] = v
                    if j + 1 == NCH:
                        for blk, signs in SIGNS.items():
                            if n in signs and all(k in order[:pos + 1] for k in signs):
                                t = v
                                for k, sg in signs.items():
                                    if k != n:
                                        t = t + acc_s[2 * k + c] if sg > 0 else t - acc_s[2 * k + c]
                                mixed(2 * blk[0] + c, blk[1], t * l_s[0, rows[blk[1]], :])

        def out_done(c, half, t):
            o_ref[half, :, lt(c)] = t.astype(o_ref.dtype)
        outs = []
        unproject(F_VO, ya_s, (1, 3, 5, 2, 4, 0, 6), False, out_done, outs)

        for pos in range(NY):
            a0, a1 = _split(HQ, NY, pos, 16)
            for c in range(2):
                blocks = [h_s[cc, half * HQ + a0:half * HQ + a1, :] for cc in (c, c + 2) for half in range(2)]
                blocks[0], blocks[3] = after(blocks[0], outs[pos][:, lt(c)]), after(blocks[3], outs[pos][:, lt(c)])
                store_operands((b + 1) % 2, h0 + a0, a1 - a0, c, blocks)

    @jax.jit
    def fn(x, w_q, w_k, w_v, w_ao, w_up, dw, w_dn, w_merge):
        B, T, D = x.shape
        K = dw.shape[0]
        HT = T // 2
        HP = (HT + HK - 1) // HK * HK
        ND = D // LN
        V = pltpu.VMEM
        out = pl.pallas_call(
            functools.partial(kernel, T=T, D=D, K=K, HP=HP),
            grid=(B, HT // HQ),
            in_specs=[pl.BlockSpec(memory_space=pl.ANY)] * 9,
            out_specs=pl.BlockSpec((None, 2, HQ, D), lambda b, i: (b, 0, i, 0)),
            out_shape=jax.ShapeDtypeStruct((B, 2, HT, D), x.dtype),
            scratch_shapes=[
                V((B, 2, HT, D), BF16),
                V((12, D, D), BF16),
                V(dw.shape, BF16),
                pltpu.SemaphoreType.DMA((10,)),
                pltpu.SemaphoreType.DMA((HT // HQ,)),
                V((5, D, D), F32),
                V((5, 7, D // 2, D // 2), BF16),
                V((28, HP, LN), BF16),
                V((K, 8, D), F32),
                V((HALO, D), F32),
                pltpu.SMEM((1,), jnp.int32),
                V((2 * ND, HQ + 2 * HALO, LN), F32),
                V((ND, TQ, LN), F32),
                V((ND, TQ, LN), F32),
                V((14, HQ, LN), BF16),
                V((ND, TQ, LN), F32),
                V((1, TQ, LN), F32),
                V((1, TQ, LN), F32),
                V((1, TQ, LN), F32),
                V((14, HQ, LN), BF16),
                V((14, HQ, LN), BF16),
                V((ND, TQ, LN), F32),
                V((2 * HP // LN, TQ, LN), F32),
                V((28, HQ, LN), BF16),
                V((14, HQ, LN), F32),
            ],
            compiler_params=pltpu.CompilerParams(
                dimension_semantics=("arbitrary", "arbitrary"),
                vmem_limit_bytes=100 * 1024 * 1024,
                flags=flags,
            ),
        )(x.reshape(B, 2, HT, D), w_q, w_k, w_v, w_ao, w_up, dw, w_dn, w_merge)
        return out.reshape(B, T, D)

    return fn


_KERNEL = make()


@jax.jit
def pallas_standalone__conformer_family_branchformer__speech_kernel(
    x: jax.Array,
    w_q: jax.Array,
    w_k: jax.Array,
    w_v: jax.Array,
    w_ao: jax.Array,
    w_up: jax.Array,
    dw: jax.Array,
    w_dn: jax.Array,
    w_merge: jax.Array,
):
    return _KERNEL(x, w_q, w_k, w_v, w_ao, w_up, dw, w_dn, w_merge)
```

```python
import functools
import math

import jax
import jax.numpy as jnp
import numpy as np
from jax import lax
import jax.experimental.pallas as pl
import jax.experimental.pallas.tpu as pltpu

F32 = jnp.float32
BF16 = jnp.bfloat16
U32 = jnp.uint32
EPS = 1e-5
LOG2E = 1.4426950408889634
HALO = 16
LN = 128


def _ln(x):
    m = jnp.mean(x, axis=-1, keepdims=True)
    xc = x - m
    v = jnp.mean(xc * xc, axis=-1, keepdims=True)
    return xc * lax.rsqrt(v + EPS)


def _gelu(x):
    c = math.sqrt(2.0 / math.pi)
    return (0.5 * x) * (1.0 + jnp.tanh(x * (c + (c * 0.044715) * (x * x))))


def _dot(a, b):
    return jnp.dot(a, b, preferred_element_type=F32)


def _dot_nt(a, b):
    return lax.dot_general(a, b, (((1,), (1,)), ((), ())), preferred_element_type=F32)


def _cat(xs):
    return jnp.concatenate(xs, axis=1)


def _spread(o, n):
    g = o.shape[0] // 8
    k = n // 8
    return jnp.concatenate([o[8 * (i * g // k):8 * (i * g // k) + 8] for i in range(k)], axis=0)


def _split(n, parts, p, unit=8):
    g = n // unit
    return unit * (p * g // parts), unit * ((p + 1) * g // parts)


def _pack(v):
    n = v.shape[0]
    v = v.reshape(n // 16, 2, 8, LN)
    return pltpu.pack_elementwise([v[:, 0].reshape(n // 2, LN), v[:, 1].reshape(n // 2, LN)], packed_dtype=BF16)


def _rows(w):
    return pltpu.bitcast(w, BF16)


def _store_shuffled(ref, k, a0, a1, v):
    n = a1 - a0
    v = v.reshape(n // 16, 2, 8, LN)
    for e in range(2):
        ref[k, pl.ds(a0 + e, n // 2, stride=2), :] = v[:, e].reshape(n // 2, LN)


def _load_unshuffled(ref, k, a0, a1):
    n = a1 - a0
    parts = [ref[k, pl.ds(a0 + e, n // 2, stride=2), :].reshape(n // 16, 1, 8, LN) for e in range(2)]
    return jnp.concatenate(parts, axis=1).reshape(n, LN)


def _left(a11, a12, a21, a22):
    return (a11 + a22, a21 + a22, a11, a22, a11 + a12, a21 - a11, a12 - a22)


def _right(b11, b12, b21, b22):
    return (b11 + b22, b11, b12 - b22, b21 - b11, b22, b11 + b12, b21 + b22)


SIGNS = {(0, 0): {0: 1, 3: 1, 4: -1, 6: 1}, (0, 1): {2: 1, 4: 1},
         (1, 0): {1: 1, 3: 1}, (1, 1): {0: 1, 1: -1, 2: 1, 5: 1}}


def _collect(order, n, v, load, store, done, opened=False):
    seen = order[:order.index(n)]
    for blk, signs in SIGNS.items():
        if n not in signs:
            continue
        if opened or any(k in signs for k in seen):
            t = load(blk) + v if signs[n] > 0 else load(blk) - v
        else:
            t = v if signs[n] > 0 else -v
        if all(k == n or k in seen for k in signs):
            done(blk, t)
        else:
            store(blk, t)


def make(HQ=400, LNT=4, NEXP=6, XA=2, FN=256, NX=6, NY=6, flags=None):
    TQ = 2 * HQ
    HK = 256

    def kernel(x_hbm, wq_hbm, wk_hbm, wv_hbm, wao_hbm, wup_hbm, dw_hbm, wdn_hbm, wm_hbm,
               o_ref,
               x_s, w_s, dw_ref, wsem, xsem,
               wf_s, wc_s, y_s, dwb_s, gb_s, z_s,
               g_s, cv_s, t_s, q_s, h_s, m_s, r_s, l_s, ya_s, yc_s, o_s, s_s, p_s, acc_s,
               *, T, D, K, HP):
        b = pl.program_id(0)
        i = pl.program_id(1)
        HT = T // 2
        HD = D // 2
        NCH = HP // HK
        ND = D // LN
        lt = lambda c: slice(c * LN, (c + 1) * LN)
        rows = (slice(0, HQ), slice(HQ, TQ))

        WAO, WV, WMA, TMP = 0, 1, 3, 4
        WDN, WMC, WQ, WK, WU, WG = 2, 6, 8, 9, 10, 11
        w_dma = [pltpu.make_async_copy(src, dst, wsem.at[n]) for n, (src, dst) in enumerate((
            (wq_hbm, w_s.at[WQ]), (wk_hbm, w_s.at[WK]), (wao_hbm, w_s.at[WAO]), (wm_hbm.at[0:D], w_s.at[WMA]),
            (wv_hbm, w_s.at[WV]), (wdn_hbm, w_s.at[WDN]), (wm_hbm.at[D:2 * D], w_s.at[WMC]),
            (dw_hbm, dw_ref), (wup_hbm.at[:, 0:D], w_s.at[WU]), (wup_hbm.at[:, D:2 * D], w_s.at[WG])))]
        F_VO, F_DC, F_QK, F_U, F_G = range(5)

        NB = x_s.shape[0]
        NI = HT // HQ

        def x_dma(bb, j):
            r = pl.ds(pl.multiple_of(j * HQ, 16), HQ)
            return pltpu.make_async_copy(x_hbm.at[bb, :, r], x_s.at[bb, :, r], xsem.at[j])

        def store_operands(slot, r, n, c, blocks):
            for k, y in enumerate(_right(*blocks)):
                y_s[14 * slot + 2 * k + c, pl.ds(r, n // 2), :] = _pack(y)

        @pl.when((b == 0) & (i == 0))
        def _():
            for n in range(4):
                w_dma[n].start()
            y_s[:, HT // 2:HP // 2, :] = jnp.zeros((y_s.shape[0], (HP - HT) // 2, LN), y_s.dtype)
            cols = lambda c: pl.ds(pl.multiple_of(c * FN, FN), FN)
            w_dma[0].wait()
            w_dma[1].wait()
            for n in range(4, 7):
                w_dma[n].start()

            def fold_qk(c, carry):
                wf_s[F_QK, :, cols(c)] = _dot_nt(w_s[WQ], w_s[WK, cols(c), :]) * (float(D) ** -0.5 * LOG2E)
                return carry
            lax.fori_loop(0, D // FN, fold_qk, 0)
            w_dma[2].wait()
            w_dma[3].wait()
            for j in range(XA):
                x_dma(0, j).start()

            def fold(t, carry):
                f, c = t // (D // FN), t % (D // FN)

                @pl.when(t == D // FN)
                def _():
                    for n in range(4, 7):
                        w_dma[n].wait()
                    for j in range(XA, NI):
                        x_dma(0, j).start()
                    for n in range(7, 10):
                        w_dma[n].start()

                rhs = jnp.where(f == 2, WMC, WMA + f)
                v = _dot(w_s[f], w_s[rhs, :, cols(c)])
                w_s[rhs + 1, :, cols(c)] = v.astype(BF16)
                wf_s[jnp.maximum(f - 1, 0), :, cols(c)] = v
                return carry
            lax.fori_loop(0, 3 * D // FN, fold, 0)
            z_s[0] = 0
            for ref in (g_s, cv_s, t_s, q_s, h_s, m_s, r_s, l_s, ya_s, yc_s, o_s, s_s, p_s, acc_s):
                ref[b, 0:16, :] = jnp.zeros((16, LN), ref.dtype)

            def first(j, carry):
                x_dma(0, j).wait()
                r = pl.multiple_of(j * HQ, 16)
                xa, xb = [_ln(x_s[0, half, pl.ds(r, HQ), :].astype(F32)) for half in range(2)]
                for c in range(2):
                    store_operands(0, pl.multiple_of(j * (HQ // 2), 8), HQ, c, (xa[:, lt(c)], xb[:, lt(c)], xa[:, lt(2 + c)], xb[:, lt(2 + c)]))
                return carry
            lax.fori_loop(0, NI, first, 0)
            if NB > 1:
                x_dma(1, 0).start()

            if True:
                for n in range(7, 10):
                    w_dma[n].wait()
                dw = dw_ref[...].astype(F32)
                for k in range(K):
                    dwb_s[k] = jnp.broadcast_to(dw[k:k + 1, :], (8, D))

                def blocks(f):
                    return (wf_s[f, 0:HD, 0:HD], wf_s[f, 0:HD, HD:D], wf_s[f, HD:D, 0:HD], wf_s[f, HD:D, HD:D])

                def right(f, carry):
                    for n, w in enumerate(_right(*blocks(f))):
                        wc_s[f, n] = pltpu.bitcast(w.astype(BF16), wc_s.dtype)
                    return carry
                lax.fori_loop(F_VO, F_QK, right, 0)

                def left(f, carry):
                    @pl.when(f > F_QK)
                    def _():
                        wf_s[f] = w_s[WU + f - F_U].astype(F32)
                    w11, w12, w21, w22 = blocks(f)
                    for n, w in enumerate(_left(w11, w21, w12, w22)):
                        wc_s[f, n] = pltpu.bitcast(w.astype(BF16), wc_s.dtype)
                    return carry
                lax.fori_loop(F_QK, F_G + 1, left, 0)

        @pl.when(i == 0)
        def _():
            x0 = jnp.concatenate([x_s[b, 0, 0:HALO, :], x_s[b, 0, HT - HALO:HT, :], x_s[b, 1, 0:HALO, :]], axis=0)
            g0 = _ln(_gelu(_dot(_ln(x0.astype(F32)).astype(BF16), w_s[WG])))
            gb_s[...] = g0[2 * HALO:3 * HALO]
            for c in range(ND):
                g_s[c, HQ:HQ + HALO, :] = jnp.zeros((HALO, LN), F32)
                g_s[c, HQ + HALO:HQ + 2 * HALO, :] = g0[0:HALO, lt(c)]
                g_s[ND + c, HQ:HQ + 2 * HALO, :] = g0[HALO:3 * HALO, lt(c)]

        @pl.when(b + 1 < NB)
        def _():
            x_dma(b + 1, i).wait()

        nxt = b * NI + i + 1

        @pl.when(nxt // NI + 1 < NB)
        def _():
            x_dma(nxt // NI + 1, nxt % NI).start()

        h0 = pl.multiple_of(i * HQ, 16)
        ys = 14 * (b % 2)
        y0 = pl.multiple_of(i * (HQ // 2), 8)
        never = lax.broadcasted_iota(jnp.int32, (8, LN), 1) < z_s[0]

        def after(v, o):
            n = v.shape[0]
            if o.shape[0] != n:
                o = _spread(o, n)
            return jnp.where(never[None], o.reshape(n // 8, 8, LN), v.reshape(n // 8, 8, LN)).reshape(n, LN)

        pair = lambda ref, n: _cat([ref[2 * n], ref[2 * n + 1]])
        ykeys = lambda n, j: _rows(_cat([y_s[ys + 2 * n + c, j * HK // 2:(j + 1) * HK // 2, :] for c in range(2)]))

        def project(f, r, ref, done, hook=None):
            order = (1, 3, 2, 4, 0, 5, 6)
            for n in order:
                mm = _dot(_rows(_cat([y_s[ys + 2 * n + c, pl.ds(r, HQ // 2), :] for c in range(2)])), _rows(wc_s[f, n]))
                for c in range(2):
                    def store(blk, t):
                        ref[2 * blk[0] + c, rows[blk[1]], :] = t
                    _collect(order, n, mm[:, lt(c)], lambda blk: ref[2 * blk[0] + c, rows[blk[1]], :], store,
                             lambda blk, t: done(2 * blk[0] + c, blk[1], t))
                if hook is not None:
                    hook(order.index(n), mm[:, lt(0)])

        def operands(dst, tmp):
            def done(c, half, t):
                if (c // 2, half) != (0, 0):
                    tmp[c, rows[half], :] = t
                else:
                    blocks = (t, tmp[c + 2, rows[0], :], tmp[c, rows[1], :], tmp[c + 2, rows[1], :])
                    for n, a in enumerate(_left(*blocks)):
                        dst[2 * n + c] = a.astype(BF16) if dst.dtype == BF16 else _pack(a)
            return done

        def carry_halo(pos, o):
            if pos < ND:
                for k in (pos, ND + pos):
                    g_s[k, 0:2 * HALO, :] = after(g_s[k, HQ:HQ + 2 * HALO, :], o)

        project(F_QK, y0, t_s, operands(q_s, t_s), carry_halo)

        def gate_done(c, half, t):
            h_s[c, rows[half], :] = _gelu(t)
        project(F_G, y0 + HALO // 2, h_s, gate_done)

        def gate_norm(half, a0, a1, o):
            n = a1 - a0
            gg = _ln(_cat([_load_unshuffled(h_s, c, half * HQ + a0, half * HQ + a1) for c in range(ND)]))
            for c in range(ND):
                gc = after(gg[:, lt(c)], o)
                k = half * ND + c
                if a1 == HQ:
                    row = lax.broadcasted_iota(jnp.int32, (HALO, LN), 0) + (h0 + HQ)
                    past = gb_s[:, lt(c)] if half == 0 else 0.0
                    g_s[k, 2 * HALO + a0:HALO + HQ, :] = gc[0:n - HALO]
                    g_s[k, HALO + HQ:2 * HALO + HQ, :] = jnp.where(row < HT, gc[n - HALO:n], past)
                else:
                    g_s[k, 2 * HALO + a0:2 * HALO + a1, :] = gc

        def conv_part(half, c, a0, a1, o):
            rc = a1 - a0
            gt = g_s[half * ND + c, a0:a1 + 2 * HALO, :].reshape((rc + 2 * HALO) // 8, 8, LN)
            acc = None
            for bb in range(8):
                n = rc // 8 + (1 if bb else 0)
                y = None
                for a in range(4):
                    k = 8 * a + bb - 1
                    if k < 0:
                        continue
                    t = gt[a:a + n] * dwb_s[k, :, lt(c)][None]
                    y = t if y is None else y + t
                y = y.reshape(n * 8, LN)[bb:bb + rc]
                acc = y if acc is None else acc + y
            _store_shuffled(cv_s, c, half * HQ + a0, half * HQ + a1, after(acc, o))

        def unproject(f, src, dst, order, first, done, results=None):
            for n in order:
                lhs = pair(src, n)
                mm = _dot(lhs if lhs.dtype == BF16 else _rows(lhs), _rows(wc_s[f, n]))
                if results is not None:
                    results.append(mm)
                for c in range(2):
                    seen = order[:order.index(n)]

                    def load(blk):
                        cc = 2 * blk[1] + c
                        if not first and not any(k in SIGNS[blk] for k in seen):
                            local = _load_unshuffled(t_s, cc, blk[0] * HQ, (blk[0] + 1) * HQ)
                            return local + x_s[b, blk[0], pl.ds(h0, HQ), lt(cc)].astype(F32)
                        return dst[cc, rows[blk[0]], :]

                    def store(blk, t):
                        dst[2 * blk[1] + c, rows[blk[0]], :] = t
                    _collect(order, n, mm[:, lt(c)], load, store,
                             (lambda blk, t: done(2 * blk[1] + c, blk[0], t)) if done else store, opened=not first)

        nslots = 7 * (NCH - 1) - LNT
        per = nslots // (2 * ND)
        order = tuple(range(7))
        for j in range(NCH):
            if j == NCH - 1:
                local = operands(yc_s, t_s)
                project(F_U, y0, t_s, lambda c, half, t: local(c, half, _gelu(t) * cv_s[c, rows[half], :]))
            for n in order:
                mm = _dot_nt(_rows(pair(q_s, n)), ykeys(n, j))
                fin = []
                for c in range(2):
                    def store(blk, t):
                        s_s[4 * j + 2 * blk[1] + c, rows[blk[0]], :] = t

                    def done(blk, t):
                        k0 = j * HK + c * LN
                        if k0 + LN > HT:
                            col = lax.broadcasted_iota(jnp.int32, t.shape, 1) + k0
                            t = jnp.where(col < HT, t, -jnp.inf)
                        store(blk, t)
                        fin.append((blk, t))
                    _collect(order, n, mm[:, lt(c)], lambda blk: s_s[4 * j + 2 * blk[1] + c, rows[blk[0]], :], store, done)
                if fin:
                    rr = rows[fin[0][0][0]]
                    mx = jnp.maximum(fin[0][1], fin[1][1])
                    m_s[0, rr, :] = mx if (j == 0 and n < 5) else jnp.maximum(mx, m_s[0, rr, :])
                t = 7 * j + n
                if t < LNT:
                    gate_norm(t % 2, *_split(HQ, LNT // 2, t // 2, 16), mm[:, lt(0)])
                elif t - LNT < per * 2 * ND:
                    k = (t - LNT) // per
                    conv_part(k % 2, k // 2, *_split(HQ, per, (t - LNT) % per, 16), mm[:, lt(0)])

        unproject(F_DC, yc_s, t_s, order, True, None)

        lane_max = m_s[0]
        m = jnp.broadcast_to(jnp.max(lane_max, axis=-1, keepdims=True), (TQ, LN))
        est = jnp.sum(jnp.exp2(lane_max - m), axis=-1, keepdims=True)
        m_s[0] = m
        r_s[0] = jnp.broadcast_to(1.0 / est, (TQ, LN))

        def exp_rows(j, a0, a1, o):
            ka, kb = 4 * j, 4 * j + 2
            rt, rb = slice(a0, a1), slice(HQ + a0, HQ + a1)
            mt, mb, st, sb = m_s[0, rt, :], m_s[0, rb, :], r_s[0, rt, :], r_s[0, rb, :]
            lt_, lb_ = None, None
            for c in range(2):
                p11 = jnp.exp2(s_s[ka + c, rt, :] - mt) * st
                p12 = jnp.exp2(s_s[kb + c, rt, :] - mt) * st
                p21 = jnp.exp2(s_s[ka + c, rb, :] - mb) * sb
                p22 = jnp.exp2(s_s[kb + c, rb, :] - mb) * sb
                if o is not None:
                    p11, p22 = after(p11, o[:, lt(c)]), after(p22, o[:, lt(c)])
                for n, p in enumerate(_right(p11, p21, p12, p22)):
                    p_s[14 * (j % 2) + 2 * n + c, a0 // 2:a1 // 2, :] = _pack(p)
                lt_ = p11 + p12 if c == 0 else lt_ + (p11 + p12)
                lb_ = p21 + p22 if c == 0 else lb_ + (p21 + p22)
            if j > 0:
                lt_, lb_ = lt_ + l_s[0, rt, :], lb_ + l_s[0, rb, :]
            if j + 1 == NCH:
                lt_, lb_ = [jnp.broadcast_to(1.0 / jnp.sum(v, axis=-1, keepdims=True), v.shape) for v in (lt_, lb_)]
                _store_shuffled(l_s, 1, a0, a1, lt_)
                _store_shuffled(l_s, 1, HQ + a0, HQ + a1, lb_)
            else:
                l_s[0, rt, :] = lt_
                l_s[0, rb, :] = lb_

        y_of = (0, 6, 1, 4, 5, 3, 2)
        order = (2, 4, 1, 3, 0, 5, 6)
        mixed = operands(ya_s, cv_s)
        exp_rows(0, 0, HQ, None)
        for j in range(NCH):
            for pos, n in enumerate(order):
                o = _dot(_rows(pair(p_s, 7 * (j % 2) + n)), ykeys(y_of[n], j))
                if j + 1 < NCH and pos < NEXP:
                    exp_rows(j + 1, *_split(HQ, NEXP, pos, 16), o)
                if j + 1 == NCH and pos < NX:
                    a0, a1 = _split(HQ, NX, pos, 16)
                    for half in range(2):
                        xn = _ln(x_s[jnp.minimum(b + 1, NB - 1), half, pl.ds(h0 + a0, a1 - a0), :].astype(F32))
                        for c in range(ND):
                            h_s[c, half * HQ + a0:half * HQ + a1, :] = after(xn[:, lt(c)], o[:, lt(half)])
                for c in range(2):
                    v = o[:, lt(c)]
                    if j > 0:
                        v = v + acc_s[2 * n + c]
                    if j + 1 < NCH or pos < 5:
                        acc_s[2 * n + c] = v
                    if j + 1 == NCH:
                        for blk, signs in SIGNS.items():
                            if n in signs and all(k in order[:pos + 1] for k in signs):
                                t = v
                                for k, sg in signs.items():
                                    if k != n:
                                        t = t + acc_s[2 * k + c] if sg > 0 else t - acc_s[2 * k + c]
                                mixed(2 * blk[0] + c, blk[1], t * l_s[1, rows[blk[1]], :])

        def out_done(c, half, t):
            o_ref[half, :, lt(c)] = t.astype(o_ref.dtype)
        outs = []
        unproject(F_VO, ya_s, o_s, (1, 3, 5, 2, 4, 0, 6), False, out_done, outs)

        for pos in range(NY):
            a0, a1 = _split(HQ, NY, pos, 16)
            for c in range(2):
                blocks = [h_s[cc, half * HQ + a0:half * HQ + a1, :] for cc in (c, c + 2) for half in range(2)]
                blocks[0], blocks[3] = after(blocks[0], outs[pos][:, lt(c)]), after(blocks[3], outs[pos][:, lt(c)])
                store_operands((b + 1) % 2, y0 + a0 // 2, a1 - a0, c, blocks)

    @jax.jit
    def fn(x, w_q, w_k, w_v, w_ao, w_up, dw, w_dn, w_merge):
        B, T, D = x.shape
        K = dw.shape[0]
        HT = T // 2
        HP = (HT + HK - 1) // HK * HK
        ND = D // LN
        V = pltpu.VMEM
        out = pl.pallas_call(
            functools.partial(kernel, T=T, D=D, K=K, HP=HP),
            grid=(B, HT // HQ),
            in_specs=[pl.BlockSpec(memory_space=pl.ANY)] * 9,
            out_specs=pl.BlockSpec((None, 2, HQ, D), lambda b, i: (b, 0, i, 0)),
            out_shape=jax.ShapeDtypeStruct((B, 2, HT, D), x.dtype),
            scratch_shapes=[
                V((B, 2, HT, D), BF16),
                V((12, D, D), BF16),
                V(dw.shape, BF16),
                pltpu.SemaphoreType.DMA((10,)),
                pltpu.SemaphoreType.DMA((HT // HQ,)),
                V((5, D, D), F32),
                V((5, 7, D // 4, D // 2), U32),
                V((28, HP // 2, LN), U32),
                V((K, 8, D), F32),
                V((HALO, D), F32),
                pltpu.SMEM((1,), jnp.int32),
                V((2 * ND, HQ + 2 * HALO, LN), F32),
                V((ND, TQ, LN), F32),
                V((ND, TQ, LN), F32),
                V((14, HQ // 2, LN), U32),
                V((ND, TQ, LN), F32),
                V((1, TQ, LN), F32),
                V((1, TQ, LN), F32),
                V((2, TQ, LN), F32),
                V((14, HQ // 2, LN), U32),
                V((14, HQ, LN), BF16),
                V((ND, TQ, LN), F32),
                V((2 * HP // LN, TQ, LN), F32),
                V((28, HQ // 2, LN), U32),
                V((14, HQ, LN), F32),
            ],
            compiler_params=pltpu.CompilerParams(
                dimension_semantics=("arbitrary", "arbitrary"),
                vmem_limit_bytes=100 * 1024 * 1024,
                flags=flags,
            ),
        )(x.reshape(B, 2, HT, D), w_q, w_k, w_v, w_ao, w_up, dw, w_dn, w_merge)
        return out.reshape(B, T, D)

    return fn


_KERNEL = make()


@jax.jit
def pallas_standalone__conformer_family_branchformer__speech_kernel(
    x: jax.Array,
    w_q: jax.Array,
    w_k: jax.Array,
    w_v: jax.Array,
    w_ao: jax.Array,
    w_up: jax.Array,
    dw: jax.Array,
    w_dn: jax.Array,
    w_merge: jax.Array,
):
    return _KERNEL(x, w_q, w_k, w_v, w_ao, w_up, dw, w_dn, w_merge)
```

```python
import functools
import math

import jax
import jax.numpy as jnp
import numpy as np
from jax import lax
import jax.experimental.pallas as pl
import jax.experimental.pallas.tpu as pltpu

F32 = jnp.float32
BF16 = jnp.bfloat16
EPS = 1e-5
LOG2E = 1.4426950408889634
HALO = 16
LN = 128


def _ln(x):
    m = jnp.mean(x, axis=-1, keepdims=True)
    xc = x - m
    v = jnp.mean(xc * xc, axis=-1, keepdims=True)
    return xc * lax.rsqrt(v + EPS)


def _gelu(x):
    c = math.sqrt(2.0 / math.pi)
    return (0.5 * x) * (1.0 + jnp.tanh(x * (c + (c * 0.044715) * (x * x))))


def _dot(a, b):
    return jnp.dot(a, b, preferred_element_type=F32)


def _dot_nt(a, b):
    return lax.dot_general(a, b, (((1,), (1,)), ((), ())), preferred_element_type=F32)


def _cat(xs):
    return jnp.concatenate(xs, axis=1)


def _spread(o, n):
    g = o.shape[0] // 8
    k = n // 8
    return jnp.concatenate([o[8 * (i * g // k):8 * (i * g // k) + 8] for i in range(k)], axis=0)


def _split(n, parts, p, unit=8):
    g = n // unit
    return unit * (p * g // parts), unit * ((p + 1) * g // parts)


def _rows(ref, k, r, n):
    return pltpu.bitcast(ref.bitcast(jnp.uint32)[k, pl.ds(r, n), :], BF16)


def _left(a11, a12, a21, a22):
    return (a11 + a22, a21 + a22, a11, a22, a11 + a12, a21 - a11, a12 - a22)


def _right(b11, b12, b21, b22):
    return (b11 + b22, b11, b12 - b22, b21 - b11, b22, b11 + b12, b21 + b22)


SIGNS = {(0, 0): {0: 1, 3: 1, 4: -1, 6: 1}, (0, 1): {2: 1, 4: 1},
         (1, 0): {1: 1, 3: 1}, (1, 1): {0: 1, 1: -1, 2: 1, 5: 1}}


def _collect(order, n, v, load, store, done, opened=False):
    seen = order[:order.index(n)]
    for blk, signs in SIGNS.items():
        if n not in signs:
            continue
        if opened or any(k in signs for k in seen):
            t = load(blk) + v if signs[n] > 0 else load(blk) - v
        else:
            t = v if signs[n] > 0 else -v
        if all(k == n or k in seen for k in signs):
            done(blk, t)
        else:
            store(blk, t)


def make(HQ=400, LNT=4, NEXP=6, XA=2, FN=256, NX=6, NY=6, flags=None):
    TQ = 2 * HQ
    HK = 256

    def kernel(x_hbm, wq_hbm, wk_hbm, wv_hbm, wao_hbm, wup_hbm, dw_hbm, wdn_hbm, wm_hbm,
               o_ref,
               x_s, w_s, dw_ref, wsem, xsem,
               wf_s, wc_s, y_s, dwb_s, gb_s, z_s,
               g_s, cv_s, t_s, q_s, h_s, m_s, r_s, l_s, ya_s, yc_s, o_s, s_s, p_s, acc_s,
               *, T, D, K, HP):
        b = pl.program_id(0)
        i = pl.program_id(1)
        HT = T // 2
        HD = D // 2
        NCH = HP // HK
        ND = D // LN
        lt = lambda c: slice(c * LN, (c + 1) * LN)
        rows = (slice(0, HQ), slice(HQ, TQ))

        WAO, WV, WMA, TMP = 0, 1, 3, 4
        WDN, WMC, WQ, WK, WU, WG = 2, 6, 8, 9, 10, 11
        w_dma = [pltpu.make_async_copy(src, dst, wsem.at[n]) for n, (src, dst) in enumerate((
            (wq_hbm, w_s.at[WQ]), (wk_hbm, w_s.at[WK]), (wao_hbm, w_s.at[WAO]), (wm_hbm.at[0:D], w_s.at[WMA]),
            (wv_hbm, w_s.at[WV]), (wdn_hbm, w_s.at[WDN]), (wm_hbm.at[D:2 * D], w_s.at[WMC]),
            (dw_hbm, dw_ref), (wup_hbm.at[:, 0:D], w_s.at[WU]), (wup_hbm.at[:, D:2 * D], w_s.at[WG])))]
        F_VO, F_DC, F_QK, F_U, F_G = range(5)

        NB = x_s.shape[0]
        NI = HT // HQ

        def x_dma(bb, j):
            r = pl.ds(pl.multiple_of(j * HQ, 16), HQ)
            return pltpu.make_async_copy(x_hbm.at[bb, :, r], x_s.at[bb, :, r], xsem.at[j])

        def store_operands(slot, r, n, c, blocks):
            for k, y in enumerate(_right(*blocks)):
                y_s[14 * slot + 2 * k + c, pl.ds(r, n), :] = y.astype(BF16)

        @pl.when((b == 0) & (i == 0))
        def _():
            for n in range(4):
                w_dma[n].start()
            y_s[:, HT:HP, :] = jnp.zeros((y_s.shape[0], HP - HT, LN), BF16)
            cols = lambda c: pl.ds(pl.multiple_of(c * FN, FN), FN)
            w_dma[0].wait()
            w_dma[1].wait()
            for n in range(4, 7):
                w_dma[n].start()

            def fold_qk(c, carry):
                wf_s[F_QK, :, cols(c)] = _dot_nt(w_s[WQ], w_s[WK, cols(c), :]) * (float(D) ** -0.5 * LOG2E)
                return carry
            lax.fori_loop(0, D // FN, fold_qk, 0)
            w_dma[2].wait()
            w_dma[3].wait()
            for j in range(XA):
                x_dma(0, j).start()

            def fold(t, carry):
                f, c = t // (D // FN), t % (D // FN)

                @pl.when(t == D // FN)
                def _():
                    for n in range(4, 7):
                        w_dma[n].wait()
                    for j in range(XA, NI):
                        x_dma(0, j).start()
                    for n in range(7, 10):
                        w_dma[n].start()

                rhs = jnp.where(f == 2, WMC, WMA + f)
                v = _dot(w_s[f], w_s[rhs, :, cols(c)])
                w_s[rhs + 1, :, cols(c)] = v.astype(BF16)
                wf_s[jnp.maximum(f - 1, 0), :, cols(c)] = v
                return carry
            lax.fori_loop(0, 3 * D // FN, fold, 0)
            z_s[0] = 0
            for ref in (g_s, cv_s, t_s, q_s, h_s, m_s, r_s, l_s, ya_s, yc_s, o_s, s_s, p_s, acc_s):
                ref[b, 0:16, :] = jnp.zeros((16, LN), ref.dtype)

            def first(j, carry):
                x_dma(0, j).wait()
                r = pl.multiple_of(j * HQ, 16)
                xa, xb = [_ln(x_s[0, half, pl.ds(r, HQ), :].astype(F32)) for half in range(2)]
                for c in range(2):
                    store_operands(0, r, HQ, c, (xa[:, lt(c)], xb[:, lt(c)], xa[:, lt(2 + c)], xb[:, lt(2 + c)]))
                return carry
            lax.fori_loop(0, NI, first, 0)
            if NB > 1:
                x_dma(1, 0).start()

            if True:
                for n in range(7, 10):
                    w_dma[n].wait()
                dw = dw_ref[...].astype(F32)
                for k in range(K):
                    dwb_s[k] = jnp.broadcast_to(dw[k:k + 1, :], (8, D))

                def blocks(f):
                    return (wf_s[f, 0:HD, 0:HD], wf_s[f, 0:HD, HD:D], wf_s[f, HD:D, 0:HD], wf_s[f, HD:D, HD:D])

                def right(f, carry):
                    for n, w in enumerate(_right(*blocks(f))):
                        for c in range(2):
                            wc_s[14 * f + 2 * n + c] = w[:, lt(c)].astype(BF16)
                    return carry
                lax.fori_loop(F_VO, F_QK, right, 0)

                def left(f, carry):
                    @pl.when(f > F_QK)
                    def _():
                        wf_s[f] = w_s[WU + f - F_U].astype(F32)
                    w11, w12, w21, w22 = blocks(f)
                    for n, w in enumerate(_left(w11, w21, w12, w22)):
                        for c in range(2):
                            wc_s[14 * f + 2 * n + c] = w[:, lt(c)].astype(BF16)
                    return carry
                lax.fori_loop(F_QK, F_G + 1, left, 0)

        @pl.when(i == 0)
        def _():
            x0 = jnp.concatenate([x_s[b, 0, 0:HALO, :], x_s[b, 0, HT - HALO:HT, :], x_s[b, 1, 0:HALO, :]], axis=0)
            g0 = _ln(_gelu(_dot(_ln(x0.astype(F32)).astype(BF16), w_s[WG])))
            gb_s[...] = g0[2 * HALO:3 * HALO]
            for c in range(ND):
                g_s[c, HQ:HQ + HALO, :] = jnp.zeros((HALO, LN), F32)
                g_s[c, HQ + HALO:HQ + 2 * HALO, :] = g0[0:HALO, lt(c)]
                g_s[ND + c, HQ:HQ + 2 * HALO, :] = g0[HALO:3 * HALO, lt(c)]

        @pl.when(b + 1 < NB)
        def _():
            x_dma(b + 1, i).wait()

        nxt = b * NI + i + 1

        @pl.when(nxt // NI + 1 < NB)
        def _():
            x_dma(nxt // NI + 1, nxt % NI).start()

        h0 = pl.multiple_of(i * HQ, 16)
        ys = 14 * (b % 2)
        y0 = pl.multiple_of(i * (HQ // 2), 8)
        never = lax.broadcasted_iota(jnp.int32, (8, LN), 1) < z_s[0]

        def after(v, o):
            n = v.shape[0]
            if o.shape[0] != n:
                o = _spread(o, n)
            return jnp.where(never[None], o.reshape(n // 8, 8, LN), v.reshape(n // 8, 8, LN)).reshape(n, LN)

        pair = lambda ref, n: _cat([_rows(ref, 2 * n + c, 0, ref.shape[1] // 2) for c in range(2)])
        ykeys = lambda n, j: _cat([_rows(y_s, ys + 2 * n + c, j * HK // 2, HK // 2) for c in range(2)])

        def project(f, r, ref, done, hook=None):
            order = (1, 3, 2, 4, 0, 5, 6)
            for n in order:
                mm = _dot(_cat([_rows(y_s, ys + 2 * n + c, r, HQ // 2) for c in range(2)]), pair(wc_s, 7 * f + n))
                for c in range(2):
                    def store(blk, t):
                        ref[2 * blk[0] + c, rows[blk[1]], :] = t
                    _collect(order, n, mm[:, lt(c)], lambda blk: ref[2 * blk[0] + c, rows[blk[1]], :], store,
                             lambda blk, t: done(2 * blk[0] + c, blk[1], t))
                if hook is not None:
                    hook(order.index(n), mm[:, lt(0)])

        def operands(dst):
            def done(c, half, t):
                if (c // 2, half) != (0, 0):
                    t_s[c, rows[half], :] = t
                else:
                    blocks = (t, t_s[c + 2, rows[0], :], t_s[c, rows[1], :], t_s[c + 2, rows[1], :])
                    for n, a in enumerate(_left(*blocks)):
                        dst[2 * n + c] = a.astype(BF16)
            return done

        def carry_halo(pos, o):
            if pos < ND:
                for k in (pos, ND + pos):
                    g_s[k, 0:2 * HALO, :] = after(g_s[k, HQ:HQ + 2 * HALO, :], o)

        project(F_QK, y0, t_s, operands(q_s), carry_halo)

        def gate_done(c, half, t):
            h_s[c, rows[half], :] = _gelu(t)
        project(F_G, y0 + HALO // 2, h_s, gate_done)

        def gate_norm(half, a0, a1, o):
            n = a1 - a0
            gg = _ln(_cat([h_s[c, half * HQ + a0:half * HQ + a1, :] for c in range(ND)]))
            for c in range(ND):
                gc = after(gg[:, lt(c)], o)
                k = half * ND + c
                if a1 == HQ:
                    row = lax.broadcasted_iota(jnp.int32, (HALO, LN), 0) + (h0 + HQ)
                    past = gb_s[:, lt(c)] if half == 0 else 0.0
                    g_s[k, 2 * HALO + a0:HALO + HQ, :] = gc[0:n - HALO]
                    g_s[k, HALO + HQ:2 * HALO + HQ, :] = jnp.where(row < HT, gc[n - HALO:n], past)
                else:
                    g_s[k, 2 * HALO + a0:2 * HALO + a1, :] = gc

        def conv_part(half, c, a0, a1, o):
            rc = a1 - a0
            gt = g_s[half * ND + c, a0:a1 + 2 * HALO, :].reshape((rc + 2 * HALO) // 8, 8, LN)
            acc = None
            for bb in range(8):
                n = rc // 8 + (1 if bb else 0)
                y = None
                for a in range(4):
                    k = 8 * a + bb - 1
                    if k < 0:
                        continue
                    t = gt[a:a + n] * dwb_s[k, :, lt(c)][None]
                    y = t if y is None else y + t
                y = y.reshape(n * 8, LN)[bb:bb + rc]
                acc = y if acc is None else acc + y
            cv_s[c, half * HQ + a0:half * HQ + a1, :] = after(acc, o)

        def unproject(f, src, order, first, done, results=None):
            for n in order:
                mm = _dot(pair(src, n), pair(wc_s, 7 * f + n))
                if results is not None:
                    results.append(mm)
                for c in range(2):
                    seen = order[:order.index(n)]

                    def load(blk):
                        cc = 2 * blk[1] + c
                        if first and not any(k in SIGNS[blk] for k in seen):
                            return x_s[b, blk[0], pl.ds(h0, HQ), lt(cc)].astype(F32)
                        return o_s[cc, rows[blk[0]], :]

                    def store(blk, t):
                        o_s[2 * blk[1] + c, rows[blk[0]], :] = t
                    _collect(order, n, mm[:, lt(c)], load, store,
                             (lambda blk, t: done(2 * blk[1] + c, blk[0], t)) if done else store, opened=True)

        nslots = 7 * (NCH - 1) - LNT
        per = nslots // (2 * ND)
        order = tuple(range(7))
        for j in range(NCH):
            if j == NCH - 1:
                local = operands(yc_s)
                project(F_U, y0, t_s, lambda c, half, t: local(c, half, _gelu(t) * cv_s[c, rows[half], :]))
            for n in order:
                mm = _dot_nt(pair(q_s, n), ykeys(n, j))
                fin = []
                for c in range(2):
                    def store(blk, t):
                        s_s[4 * j + 2 * blk[1] + c, rows[blk[0]], :] = t

                    def done(blk, t):
                        k0 = j * HK + c * LN
                        if k0 + LN > HT:
                            col = lax.broadcasted_iota(jnp.int32, t.shape, 1) + k0
                            t = jnp.where(col < HT, t, -jnp.inf)
                        store(blk, t)
                        fin.append((blk, t))
                    _collect(order, n, mm[:, lt(c)], lambda blk: s_s[4 * j + 2 * blk[1] + c, rows[blk[0]], :], store, done)
                if fin:
                    rr = rows[fin[0][0][0]]
                    mx = jnp.maximum(fin[0][1], fin[1][1])
                    m_s[0, rr, :] = mx if (j == 0 and n < 5) else jnp.maximum(mx, m_s[0, rr, :])
                t = 7 * j + n
                if t < LNT:
                    gate_norm(t % 2, *_split(HQ, LNT // 2, t // 2), mm[:, lt(0)])
                elif t - LNT < per * 2 * ND:
                    k = (t - LNT) // per
                    conv_part(k % 2, k // 2, *_split(HQ, per, (t - LNT) % per), mm[:, lt(0)])

        unproject(F_DC, yc_s, order, True, None)

        lane_max = m_s[0]
        m = jnp.broadcast_to(jnp.max(lane_max, axis=-1, keepdims=True), (TQ, LN))
        est = jnp.sum(jnp.exp2(lane_max - m), axis=-1, keepdims=True)
        m_s[0] = m
        r_s[0] = jnp.broadcast_to(1.0 / est, (TQ, LN))

        def exp_rows(j, a0, a1, o):
            ka, kb = 4 * j, 4 * j + 2
            rt, rb = slice(a0, a1), slice(HQ + a0, HQ + a1)
            mt, mb, st, sb = m_s[0, rt, :], m_s[0, rb, :], r_s[0, rt, :], r_s[0, rb, :]
            lt_, lb_ = None, None
            for c in range(2):
                p11 = jnp.exp2(s_s[ka + c, rt, :] - mt) * st
                p12 = jnp.exp2(s_s[kb + c, rt, :] - mt) * st
                p21 = jnp.exp2(s_s[ka + c, rb, :] - mb) * sb
                p22 = jnp.exp2(s_s[kb + c, rb, :] - mb) * sb
                if o is not None:
                    p11, p22 = after(p11, o[:, lt(c)]), after(p22, o[:, lt(c)])
                for n, p in enumerate(_right(p11, p21, p12, p22)):
                    p_s[14 * (j % 2) + 2 * n + c, rt, :] = p.astype(BF16)
                lt_ = p11 + p12 if c == 0 else lt_ + (p11 + p12)
                lb_ = p21 + p22 if c == 0 else lb_ + (p21 + p22)
            if j > 0:
                lt_, lb_ = lt_ + l_s[0, rt, :], lb_ + l_s[0, rb, :]
            if j + 1 == NCH:
                lt_, lb_ = [jnp.broadcast_to(1.0 / jnp.sum(v, axis=-1, keepdims=True), v.shape) for v in (lt_, lb_)]
            l_s[0, rt, :] = lt_
            l_s[0, rb, :] = lb_

        y_of = (0, 6, 1, 4, 5, 3, 2)
        order = (2, 4, 1, 3, 0, 5, 6)
        mixed = operands(ya_s)
        exp_rows(0, 0, HQ, None)
        for j in range(NCH):
            for pos, n in enumerate(order):
                o = _dot(pair(p_s, 7 * (j % 2) + n), ykeys(y_of[n], j))
                if j + 1 < NCH and pos < NEXP:
                    exp_rows(j + 1, *_split(HQ, NEXP, pos, 16), o)
                if j + 1 == NCH and pos < NX:
                    a0, a1 = _split(HQ, NX, pos, 16)
                    for half in range(2):
                        xn = _ln(x_s[jnp.minimum(b + 1, NB - 1), half, pl.ds(h0 + a0, a1 - a0), :].astype(F32))
                        for c in range(ND):
                            h_s[c, half * HQ + a0:half * HQ + a1, :] = after(xn[:, lt(c)], o[:, lt(half)])
                for c in range(2):
                    v = o[:, lt(c)]
                    if j > 0:
                        v = v + acc_s[2 * n + c]
                    if j + 1 < NCH or pos < 5:
                        acc_s[2 * n + c] = v
                    if j + 1 == NCH:
                        for blk, signs in SIGNS.items():
                            if n in signs and all(k in order[:pos + 1] for k in signs):
                                t = v
                                for k, sg in signs.items():
                                    if k != n:
                                        t = t + acc_s[2 * k + c] if sg > 0 else t - acc_s[2 * k + c]
                                mixed(2 * blk[0] + c, blk[1], t * l_s[0, rows[blk[1]], :])

        def out_done(c, half, t):
            o_ref[half, :, lt(c)] = t.astype(o_ref.dtype)
        outs = []
        unproject(F_VO, ya_s, (1, 3, 5, 2, 4, 0, 6), False, out_done, outs)

        for pos in range(NY):
            a0, a1 = _split(HQ, NY, pos, 16)
            for c in range(2):
                blocks = [h_s[cc, half * HQ + a0:half * HQ + a1, :] for cc in (c, c + 2) for half in range(2)]
                blocks[0], blocks[3] = after(blocks[0], outs[pos][:, lt(c)]), after(blocks[3], outs[pos][:, lt(c)])
                store_operands((b + 1) % 2, h0 + a0, a1 - a0, c, blocks)

    @jax.jit
    def fn(x, w_q, w_k, w_v, w_ao, w_up, dw, w_dn, w_merge):
        B, T, D = x.shape
        K = dw.shape[0]
        HT = T // 2
        HP = (HT + HK - 1) // HK * HK
        ND = D // LN
        V = pltpu.VMEM
        out = pl.pallas_call(
            functools.partial(kernel, T=T, D=D, K=K, HP=HP),
            grid=(B, HT // HQ),
            in_specs=[pl.BlockSpec(memory_space=pl.ANY)] * 9,
            out_specs=pl.BlockSpec((None, 2, HQ, D), lambda b, i: (b, 0, i, 0)),
            out_shape=jax.ShapeDtypeStruct((B, 2, HT, D), x.dtype),
            scratch_shapes=[
                V((B, 2, HT, D), BF16),
                V((12, D, D), BF16),
                V(dw.shape, BF16),
                pltpu.SemaphoreType.DMA((10,)),
                pltpu.SemaphoreType.DMA((HT // HQ,)),
                V((5, D, D), F32),
                V((70, D // 2, LN), BF16),
                V((28, HP, LN), BF16),
                V((K, 8, D), F32),
                V((HALO, D), F32),
                pltpu.SMEM((1,), jnp.int32),
                V((2 * ND, HQ + 2 * HALO, LN), F32),
                V((ND, TQ, LN), F32),
                V((ND, TQ, LN), F32),
                V((14, HQ, LN), BF16),
                V((ND, TQ, LN), F32),
                V((1, TQ, LN), F32),
                V((1, TQ, LN), F32),
                V((1, TQ, LN), F32),
                V((14, HQ, LN), BF16),
                V((14, HQ, LN), BF16),
                V((ND, TQ, LN), F32),
                V((2 * HP // LN, TQ, LN), F32),
                V((28, HQ, LN), BF16),
                V((14, HQ, LN), F32),
            ],
            compiler_params=pltpu.CompilerParams(
                dimension_semantics=("arbitrary", "arbitrary"),
                vmem_limit_bytes=100 * 1024 * 1024,
                flags=flags,
            ),
        )(x.reshape(B, 2, HT, D), w_q, w_k, w_v, w_ao, w_up, dw, w_dn, w_merge)
        return out.reshape(B, T, D)

    return fn


_KERNEL = make()


@jax.jit
def pallas_standalone__conformer_family_branchformer__speech_kernel(
    x: jax.Array,
    w_q: jax.Array,
    w_k: jax.Array,
    w_v: jax.Array,
    w_ao: jax.Array,
    w_up: jax.Array,
    dw: jax.Array,
    w_dn: jax.Array,
    w_merge: jax.Array,
):
    return _KERNEL(x, w_q, w_k, w_v, w_ao, w_up, dw, w_dn, w_merge)
```

```python
import math

import jax
import jax.numpy as jnp
from jax import lax
import jax.experimental.pallas as pl
import jax.experimental.pallas.tpu as pltpu

F32 = jnp.float32
BF16 = jnp.bfloat16
EPS = 1e-5
LOG2E = 1.4426950408889634
LANES = 128
HALO = 16
HQ = 400
HK = 256
NORM_SLOTS = 8
EXP_SLOTS = 5
NEXT_SLOTS = 6


def _ln(x):
    m = jnp.mean(x, axis=-1, keepdims=True)
    xc = x - m
    v = jnp.mean(xc * xc, axis=-1, keepdims=True)
    return xc * lax.rsqrt(v + EPS)


def _gelu(x):
    c = math.sqrt(2.0 / math.pi)
    return (0.5 * x) * (1.0 + jnp.tanh(x * (c + (c * 0.044715) * (x * x))))


def _dot(a, b):
    return jnp.dot(a, b, preferred_element_type=F32)


def _dot_nt(a, b):
    return lax.dot_general(a, b, (((1,), (1,)), ((), ())), preferred_element_type=F32)


def _cat(xs):
    return jnp.concatenate(xs, axis=1)


def _lanes(c):
    return slice(c * LANES, (c + 1) * LANES)


def _split(n, parts, p, unit=8):
    g = n // unit
    return unit * (p * g // parts), unit * ((p + 1) * g // parts)


def _spread(o, n):
    g = o.shape[0] // 8
    k = n // 8
    return jnp.concatenate([o[8 * (i * g // k):8 * (i * g // k) + 8] for i in range(k)], axis=0)


def _rows(ref, k, r, n):
    return pltpu.bitcast(ref.bitcast(jnp.uint32)[k, pl.ds(r, n), :], BF16)


def _left(a11, a12, a21, a22):
    return (a11 + a22, a21 + a22, a11, a22, a11 + a12, a21 - a11, a12 - a22)


def _right(b11, b12, b21, b22):
    return (b11 + b22, b11, b12 - b22, b21 - b11, b22, b11 + b12, b21 + b22)


SIGNS = {(0, 0): {0: 1, 3: 1, 4: -1, 6: 1}, (0, 1): {2: 1, 4: 1},
         (1, 0): {1: 1, 3: 1}, (1, 1): {0: 1, 1: -1, 2: 1, 5: 1}}


def _collect(order, n, v, load, store, done, opened=False):
    seen = order[:order.index(n)]
    for blk, signs in SIGNS.items():
        if n not in signs:
            continue
        if opened or any(k in signs for k in seen):
            t = load(blk) + v if signs[n] > 0 else load(blk) - v
        else:
            t = v if signs[n] > 0 else -v
        if all(k == n or k in seen for k in signs):
            done(blk, t)
        else:
            store(blk, t)


WAO, WV, WDN, WMA, WMC, WQ, WK, WU, WG = 0, 1, 2, 3, 6, 8, 9, 10, 11
F_VO, F_DC, F_QK, F_U, F_G = range(5)


def _kernel(x_hbm, wq_hbm, wk_hbm, wv_hbm, wao_hbm, wup_hbm, dw_hbm, wdn_hbm, wm_hbm,
            o_ref,
            x_s, w_s, dw_s, wsem, xsem,
            wf_s, wc_s, y_s, dwb_s, gb_s, zero_s,
            g_s, cv_s, t_s, q_s, h_s, m_s, r_s, l_s, ya_s, yc_s, o_s, s_s, p_s, acc_s):
    b = pl.program_id(0)
    i = pl.program_id(1)
    NB, _, HT, D = x_s.shape
    K = dw_s.shape[0]
    HD = D // 2
    ND = D // LANES
    NI = HT // HQ
    NCH = y_s.shape[1] // HK
    rows = (slice(0, HQ), slice(HQ, 2 * HQ))

    w_dma = [pltpu.make_async_copy(src, dst, wsem.at[n]) for n, (src, dst) in enumerate((
        (wq_hbm, w_s.at[WQ]), (wk_hbm, w_s.at[WK]), (wao_hbm, w_s.at[WAO]), (wm_hbm.at[0:D], w_s.at[WMA]),
        (wv_hbm, w_s.at[WV]), (wdn_hbm, w_s.at[WDN]), (wm_hbm.at[D:2 * D], w_s.at[WMC]),
        (dw_hbm, dw_s), (wup_hbm.at[:, 0:D], w_s.at[WU]), (wup_hbm.at[:, D:2 * D], w_s.at[WG])))]

    def x_dma(bb, j):
        r = pl.ds(pl.multiple_of(j * HQ, 16), HQ)
        return pltpu.make_async_copy(x_hbm.at[bb, :, r], x_s.at[bb, :, r], xsem.at[j])

    def store_keys(slot, r, n, c, blocks):
        for k, y in enumerate(_right(*blocks)):
            y_s[14 * slot + 2 * k + c, pl.ds(r, n), :] = y.astype(BF16)

    @pl.when((b == 0) & (i == 0))
    def _():
        for n in range(4):
            w_dma[n].start()
        y_s[:, HT:NCH * HK, :] = jnp.zeros((y_s.shape[0], NCH * HK - HT, LANES), BF16)
        cols = lambda c: pl.ds(pl.multiple_of(c * HD, HD), HD)
        w_dma[0].wait()
        w_dma[1].wait()
        for n in range(4, 7):
            w_dma[n].start()

        def fold_qk(c, carry):
            wf_s[F_QK, :, cols(c)] = _dot_nt(w_s[WQ], w_s[WK, cols(c), :]) * (float(D) ** -0.5 * LOG2E)
            return carry
        lax.fori_loop(0, 2, fold_qk, 0)
        w_dma[2].wait()
        w_dma[3].wait()
        for j in range(2):
            x_dma(0, j).start()

        def fold(t, carry):
            f, c = t // 2, t % 2

            @pl.when(t == 2)
            def _():
                for n in range(4, 7):
                    w_dma[n].wait()
                for j in range(2, NI):
                    x_dma(0, j).start()
                for n in range(7, 10):
                    w_dma[n].start()

            rhs = jnp.where(f == 2, WMC, WMA + f)
            v = _dot(w_s[f], w_s[rhs, :, cols(c)])
            w_s[rhs + 1, :, cols(c)] = v.astype(BF16)
            wf_s[jnp.maximum(f - 1, 0), :, cols(c)] = v
            return carry
        lax.fori_loop(0, 6, fold, 0)
        zero_s[0] = 0
        for ref in (g_s, cv_s, t_s, q_s, h_s, m_s, r_s, l_s, ya_s, yc_s, o_s, s_s, p_s, acc_s):
            ref[b, 0:16, :] = jnp.zeros((16, LANES), ref.dtype)

        def first_keys(j, carry):
            x_dma(0, j).wait()
            r = pl.multiple_of(j * HQ, 16)
            xa, xb = [_ln(x_s[0, half, pl.ds(r, HQ), :].astype(F32)) for half in range(2)]
            for c in range(2):
                store_keys(0, r, HQ, c, (xa[:, _lanes(c)], xb[:, _lanes(c)], xa[:, _lanes(2 + c)], xb[:, _lanes(2 + c)]))
            return carry
        lax.fori_loop(0, NI, first_keys, 0)
        if NB > 1:
            x_dma(1, 0).start()

        for n in range(7, 10):
            w_dma[n].wait()
        dw = dw_s[...].astype(F32)
        for k in range(K):
            dwb_s[k] = jnp.broadcast_to(dw[k:k + 1, :], (8, D))

        def blocks(f):
            return (wf_s[f, 0:HD, 0:HD], wf_s[f, 0:HD, HD:D], wf_s[f, HD:D, 0:HD], wf_s[f, HD:D, HD:D])

        def store_weights(f, operands):
            for n, w in enumerate(operands):
                for c in range(2):
                    wc_s[14 * f + 2 * n + c] = w[:, _lanes(c)].astype(BF16)

        def right(f, carry):
            store_weights(f, _right(*blocks(f)))
            return carry
        lax.fori_loop(F_VO, F_QK, right, 0)

        def left(f, carry):
            @pl.when(f > F_QK)
            def _():
                wf_s[f] = w_s[WU + f - F_U].astype(F32)
            w11, w12, w21, w22 = blocks(f)
            store_weights(f, _left(w11, w21, w12, w22))
            return carry
        lax.fori_loop(F_QK, F_G + 1, left, 0)

    @pl.when(i == 0)
    def _():
        x0 = jnp.concatenate([x_s[b, 0, 0:HALO, :], x_s[b, 0, HT - HALO:HT, :], x_s[b, 1, 0:HALO, :]], axis=0)
        g0 = _ln(_gelu(_dot(_ln(x0.astype(F32)).astype(BF16), w_s[WG])))
        gb_s[...] = g0[2 * HALO:3 * HALO]
        for c in range(ND):
            g_s[c, HQ:HQ + HALO, :] = jnp.zeros((HALO, LANES), F32)
            g_s[c, HQ + HALO:HQ + 2 * HALO, :] = g0[0:HALO, _lanes(c)]
            g_s[ND + c, HQ:HQ + 2 * HALO, :] = g0[HALO:3 * HALO, _lanes(c)]

    @pl.when(b + 1 < NB)
    def _():
        x_dma(b + 1, i).wait()

    nxt = b * NI + i + 1

    @pl.when(nxt // NI + 1 < NB)
    def _():
        x_dma(nxt // NI + 1, nxt % NI).start()

    h0 = pl.multiple_of(i * HQ, 16)
    y0 = pl.multiple_of(i * (HQ // 2), 8)
    keys = 14 * (b % 2)
    never = lax.broadcasted_iota(jnp.int32, (8, LANES), 1) < zero_s[0]

    def after(v, o):
        n = v.shape[0]
        if o.shape[0] != n:
            o = _spread(o, n)
        shape = (n // 8, 8, LANES)
        return jnp.where(never[None], o.reshape(shape), v.reshape(shape)).reshape(n, LANES)

    pair = lambda ref, n: _cat([_rows(ref, 2 * n + c, 0, ref.shape[1] // 2) for c in range(2)])
    chunk = lambda n, j: _cat([_rows(y_s, keys + 2 * n + c, j * HK // 2, HK // 2) for c in range(2)])

    def project(f, r, ref, done, hook=None):
        order = (1, 3, 2, 4, 0, 5, 6)
        for n in order:
            mm = _dot(_cat([_rows(y_s, keys + 2 * n + c, r, HQ // 2) for c in range(2)]), pair(wc_s, 7 * f + n))
            for c in range(2):
                def load(blk):
                    return ref[2 * blk[0] + c, rows[blk[1]], :]

                def store(blk, t):
                    ref[2 * blk[0] + c, rows[blk[1]], :] = t
                _collect(order, n, mm[:, _lanes(c)], load, store, lambda blk, t: done(2 * blk[0] + c, blk[1], t))
            if hook is not None:
                hook(order.index(n), mm[:, _lanes(0)])

    def merge(f, src, order, first, done):
        results = []
        for n in order:
            mm = _dot(pair(src, n), pair(wc_s, 7 * f + n))
            results.append(mm)
            seen = order[:order.index(n)]
            for c in range(2):
                def load(blk):
                    cc = 2 * blk[1] + c
                    if first and not any(k in SIGNS[blk] for k in seen):
                        return x_s[b, blk[0], pl.ds(h0, HQ), _lanes(cc)].astype(F32)
                    return o_s[cc, rows[blk[0]], :]

                def store(blk, t):
                    o_s[2 * blk[1] + c, rows[blk[0]], :] = t
                _collect(order, n, mm[:, _lanes(c)], load, store,
                         (lambda blk, t: done(2 * blk[1] + c, blk[0], t)) if done else store, opened=True)
        return results

    def operands(dst):
        def done(c, half, t):
            if (c // 2, half) != (0, 0):
                t_s[c, rows[half], :] = t
            else:
                blocks = (t, t_s[c + 2, rows[0], :], t_s[c, rows[1], :], t_s[c + 2, rows[1], :])
                for n, a in enumerate(_left(*blocks)):
                    dst[2 * n + c] = a.astype(BF16)
        return done

    def carry_halo(pos, o):
        if pos < ND:
            for k in (pos, ND + pos):
                g_s[k, 0:2 * HALO, :] = after(g_s[k, HQ:HQ + 2 * HALO, :], o)

    def gate_done(c, half, t):
        h_s[c, rows[half], :] = _gelu(t)

    def gate_norm(half, a0, a1, o):
        n = a1 - a0
        gg = _ln(_cat([h_s[c, half * HQ + a0:half * HQ + a1, :] for c in range(ND)]))
        for c in range(ND):
            gc = after(gg[:, _lanes(c)], o)
            k = half * ND + c
            if a1 == HQ:
                row = lax.broadcasted_iota(jnp.int32, (HALO, LANES), 0) + (h0 + HQ)
                past_end = gb_s[:, _lanes(c)] if half == 0 else 0.0
                g_s[k, 2 * HALO + a0:HALO + HQ, :] = gc[0:n - HALO]
                g_s[k, HALO + HQ:2 * HALO + HQ, :] = jnp.where(row < HT, gc[n - HALO:n], past_end)
            else:
                g_s[k, 2 * HALO + a0:2 * HALO + a1, :] = gc

    def conv(half, c, a0, a1, o):
        n = a1 - a0
        gt = g_s[half * ND + c, a0:a1 + 2 * HALO, :].reshape((n + 2 * HALO) // 8, 8, LANES)
        acc = None
        for shift in range(8):
            groups = n // 8 + (1 if shift else 0)
            y = None
            for a in range(2 * HALO // 8):
                k = 8 * a + shift - (HALO - K // 2)
                if 0 <= k < K:
                    t = gt[a:a + groups] * dwb_s[k, :, _lanes(c)][None]
                    y = t if y is None else y + t
            y = y.reshape(groups * 8, LANES)[shift:shift + n]
            acc = y if acc is None else acc + y
        cv_s[c, half * HQ + a0:half * HQ + a1, :] = after(acc, o)

    project(F_QK, y0, t_s, operands(q_s), carry_halo)
    project(F_G, y0 + HALO // 2, h_s, gate_done)

    per = (7 * (NCH - 1) - NORM_SLOTS) // (2 * ND)
    order = tuple(range(7))
    for j in range(NCH):
        if j == NCH - 1:
            local = operands(yc_s)
            project(F_U, y0, t_s, lambda c, half, t: local(c, half, _gelu(t) * cv_s[c, rows[half], :]))
        for n in order:
            mm = _dot_nt(pair(q_s, n), chunk(n, j))
            finished = []
            for c in range(2):
                def load(blk):
                    return s_s[4 * j + 2 * blk[1] + c, rows[blk[0]], :]

                def store(blk, t):
                    s_s[4 * j + 2 * blk[1] + c, rows[blk[0]], :] = t

                def done(blk, t):
                    k0 = j * HK + c * LANES
                    if k0 + LANES > HT:
                        col = lax.broadcasted_iota(jnp.int32, t.shape, 1) + k0
                        t = jnp.where(col < HT, t, -jnp.inf)
                    store(blk, t)
                    finished.append((blk, t))
                _collect(order, n, mm[:, _lanes(c)], load, store, done)
            if finished:
                rr = rows[finished[0][0][0]]
                mx = jnp.maximum(finished[0][1], finished[1][1])
                m_s[0, rr, :] = mx if (j == 0 and n < 5) else jnp.maximum(mx, m_s[0, rr, :])
            t = 7 * j + n
            if t < NORM_SLOTS:
                gate_norm(t % 2, *_split(HQ, NORM_SLOTS // 2, t // 2), mm[:, _lanes(0)])
            elif t - NORM_SLOTS < per * 2 * ND:
                k = (t - NORM_SLOTS) // per
                conv(k % 2, k // 2, *_split(HQ, per, (t - NORM_SLOTS) % per), mm[:, _lanes(0)])

    merge(F_DC, yc_s, order, True, None)

    lane_max = m_s[0]
    m = jnp.broadcast_to(jnp.max(lane_max, axis=-1, keepdims=True), lane_max.shape)
    bound = jnp.sum(jnp.exp2(lane_max - m), axis=-1, keepdims=True)
    m_s[0] = m
    r_s[0] = jnp.broadcast_to(1.0 / bound, lane_max.shape)

    def probabilities(j, a0, a1, o):
        ka, kb = 4 * j, 4 * j + 2
        rt, rb = slice(a0, a1), slice(HQ + a0, HQ + a1)
        mt, mb, st, sb = m_s[0, rt, :], m_s[0, rb, :], r_s[0, rt, :], r_s[0, rb, :]
        lt, lb = None, None
        for c in range(2):
            p11 = jnp.exp2(s_s[ka + c, rt, :] - mt) * st
            p12 = jnp.exp2(s_s[kb + c, rt, :] - mt) * st
            p21 = jnp.exp2(s_s[ka + c, rb, :] - mb) * sb
            p22 = jnp.exp2(s_s[kb + c, rb, :] - mb) * sb
            if o is not None:
                p11, p22 = after(p11, o[:, _lanes(c)]), after(p22, o[:, _lanes(c)])
            for n, p in enumerate(_right(p11, p21, p12, p22)):
                p_s[14 * (j % 2) + 2 * n + c, rt, :] = p.astype(BF16)
            lt = p11 + p12 if c == 0 else lt + (p11 + p12)
            lb = p21 + p22 if c == 0 else lb + (p21 + p22)
        if j > 0:
            lt, lb = lt + l_s[0, rt, :], lb + l_s[0, rb, :]
        if j + 1 == NCH:
            lt, lb = [jnp.broadcast_to(1.0 / jnp.sum(v, axis=-1, keepdims=True), v.shape) for v in (lt, lb)]
        l_s[0, rt, :] = lt
        l_s[0, rb, :] = lb

    y_of = (0, 6, 1, 4, 5, 3, 2)
    order = (2, 4, 1, 3, 0, 5, 6)
    mixed = operands(ya_s)
    probabilities(0, 0, HQ, None)
    for j in range(NCH):
        for pos, n in enumerate(order):
            o = _dot(pair(p_s, 7 * (j % 2) + n), chunk(y_of[n], j))
            if j + 1 < NCH and pos < EXP_SLOTS:
                probabilities(j + 1, *_split(HQ, EXP_SLOTS, pos, 16), o)
            if j + 1 == NCH and pos < NEXT_SLOTS:
                a0, a1 = _split(HQ, NEXT_SLOTS, pos, 16)
                for half in range(2):
                    xn = _ln(x_s[jnp.minimum(b + 1, NB - 1), half, pl.ds(h0 + a0, a1 - a0), :].astype(F32))
                    for c in range(ND):
                        h_s[c, half * HQ + a0:half * HQ + a1, :] = after(xn[:, _lanes(c)], o[:, _lanes(half)])
            for c in range(2):
                v = o[:, _lanes(c)]
                if j > 0:
                    v = v + acc_s[2 * n + c]
                if j + 1 < NCH or pos < 5:
                    acc_s[2 * n + c] = v
                if j + 1 == NCH:
                    for blk, signs in SIGNS.items():
                        if n in signs and all(k in order[:pos + 1] for k in signs):
                            t = v
                            for k, sign in signs.items():
                                if k != n:
                                    t = t + acc_s[2 * k + c] if sign > 0 else t - acc_s[2 * k + c]
                            mixed(2 * blk[0] + c, blk[1], t * l_s[0, rows[blk[1]], :])

    def out_done(c, half, t):
        o_ref[half, :, _lanes(c)] = t.astype(o_ref.dtype)
    outs = merge(F_VO, ya_s, (1, 3, 5, 2, 4, 0, 6), False, out_done)

    for pos in range(NEXT_SLOTS):
        a0, a1 = _split(HQ, NEXT_SLOTS, pos, 16)
        for c in range(2):
            blocks = [h_s[cc, half * HQ + a0:half * HQ + a1, :] for cc in (c, c + 2) for half in range(2)]
            o = outs[pos][:, _lanes(c)]
            blocks[0], blocks[3] = after(blocks[0], o), after(blocks[3], o)
            store_keys((b + 1) % 2, h0 + a0, a1 - a0, c, blocks)


@jax.jit
def pallas_standalone__conformer_family_branchformer__speech_kernel(
    x: jax.Array,
    w_q: jax.Array,
    w_k: jax.Array,
    w_v: jax.Array,
    w_ao: jax.Array,
    w_up: jax.Array,
    dw: jax.Array,
    w_dn: jax.Array,
    w_merge: jax.Array,
):
    B, T, D = x.shape
    K = dw.shape[0]
    HT = T // 2
    assert D == 4 * LANES and T % (2 * HQ) == 0 and HT >= 2 * HQ and K % 2 == 1 and K // 2 < HALO
    HP = pl.cdiv(HT, HK) * HK
    ND = D // LANES
    TQ = 2 * HQ
    vmem = pltpu.VMEM
    out = pl.pallas_call(
        _kernel,
        grid=(B, HT // HQ),
        in_specs=[pl.BlockSpec(memory_space=pl.ANY)] * 9,
        out_specs=pl.BlockSpec((None, 2, HQ, D), lambda b, i: (b, 0, i, 0)),
        out_shape=jax.ShapeDtypeStruct((B, 2, HT, D), x.dtype),
        scratch_shapes=[
            vmem((B, 2, HT, D), BF16),
            vmem((12, D, D), BF16),
            vmem((K, D), BF16),
            pltpu.SemaphoreType.DMA((10,)),
            pltpu.SemaphoreType.DMA((HT // HQ,)),
            vmem((5, D, D), F32),
            vmem((70, D // 2, LANES), BF16),
            vmem((28, HP, LANES), BF16),
            vmem((K, 8, D), F32),
            vmem((HALO, D), F32),
            pltpu.SMEM((1,), jnp.int32),
            vmem((2 * ND, HQ + 2 * HALO, LANES), F32),
            vmem((ND, TQ, LANES), F32),
            vmem((ND, TQ, LANES), F32),
            vmem((14, HQ, LANES), BF16),
            vmem((ND, TQ, LANES), F32),
            vmem((1, TQ, LANES), F32),
            vmem((1, TQ, LANES), F32),
            vmem((1, TQ, LANES), F32),
            vmem((14, HQ, LANES), BF16),
            vmem((14, HQ, LANES), BF16),
            vmem((ND, TQ, LANES), F32),
            vmem((2 * HP // LANES, TQ, LANES), F32),
            vmem((28, HQ, LANES), BF16),
            vmem((14, HQ, LANES), F32),
        ],
        compiler_params=pltpu.CompilerParams(
            dimension_semantics=("arbitrary", "arbitrary"),
            vmem_limit_bytes=100 * 1024 * 1024,
        ),
    )(x.reshape(B, 2, HT, D), w_q, w_k, w_v, w_ao, w_up, dw, w_dn, w_merge)
    return out.reshape(B, T, D)
```
